```python
import jax
import jax.numpy as jnp

def _softmax(x, axis=-1):
    return jax.nn.softmax(x, axis=axis)

def _gelu(x):
    return jax.nn.gelu(x, approximate=True)

def _silu(x):
    return jax.nn.silu(x)

def _sigmoid(x):
    return jax.nn.sigmoid(x)

def _layernorm(x, axis=-1, eps=1e-05):
    m = jnp.mean(x, axis=axis, keepdims=True)
    v = jnp.var(x, axis=axis, keepdims=True)
    return (x - m) / jnp.sqrt(v + eps)

def _scatter_add(tgt, idx, src, axis=0):
    return tgt.at[idx].add(src)

def _segment_sum(src, seg, n):
    return jax.ops.segment_sum(src, seg, n)

class _Rng:

    def __init__(self, key):
        self._k = key

    def _next(self):
        self._k, sub = jax.random.split(self._k)
        return sub

    def normal(self, shape):
        return jax.random.normal(self._next(), shape, dtype=jnp.bfloat16)

    def randint(self, lo, hi, shape):
        return jax.random.randint(self._next(), shape, lo, hi, dtype=jnp.int32)

    def uniform(self, shape, lo=0.0, hi=1.0):
        return jax.random.uniform(self._next(), shape, jnp.bfloat16, lo, hi)

    def permutation(self, n):
        return jax.random.permutation(self._next(), n)
kernel_name = 'concat_heads__softmax_full_mha__memory_aug_recurrent_mem_tr__prompt'

def setup_inputs():
    _rng = _Rng(jax.random.key(int.from_bytes(__import__("os").urandom(4), "little")))
    _w = lambda a: (lambda t: t.astype(jnp.bfloat16) if jnp.issubdtype(t.dtype, jnp.floating) else t)(jnp.asarray(a))

    def _A_setup():
        B, S, D = (1, 2048, 1024)
        return {'x': _w((lambda *s: _rng.normal(s) * 0.05)(B, S, D)), 'wqkv': _w((lambda *s: _rng.normal(s) * 0.05)(D, 3 * D)), 'wo': _w((lambda *s: _rng.normal(s) * 0.05)(D, D))}
    _A_in = _A_setup()

    def _B_setup():
        B, S, Dm = (1, 2048, 1024)
        H, Dh = (32, 128)
        M, seg = (8, 32)
        seg = min(seg, S)
        S = S // seg * seg
        return {'x': _w((lambda *s: _rng.normal(s) * 0.05)(B, S, Dm)), 'mem0': _w((lambda *s: _rng.normal(s) * 0.05)(B, M, Dm)), 'Wq': _w((lambda *s: _rng.normal(s) * 0.05)(Dm, H, Dh) * Dm ** (-0.5)), 'Wk': _w((lambda *s: _rng.normal(s) * 0.05)(Dm, H, Dh) * Dm ** (-0.5)), 'Wv': _w((lambda *s: _rng.normal(s) * 0.05)(Dm, H, Dh) * Dm ** (-0.5)), 'Wo': _w((lambda *s: _rng.normal(s) * 0.05)(H, Dh, Dm) * (H * Dh) ** (-0.5)), 'seg_len': seg}
    _B_in = _B_setup()
    return {'A_x': _A_in['x'], 'A_wqkv': _A_in['wqkv'], 'A_wo': _A_in['wo'], 'B_x': _B_in['x'], 'B_mem0': _B_in['mem0'], 'B_Wq': _B_in['Wq'], 'B_Wk': _B_in['Wk'], 'B_Wv': _B_in['Wv'], 'B_Wo': _B_in['Wo'], 'B_seg_len': _B_in['seg_len']}

def reference(A_x, A_wqkv, A_wo, B_x, B_mem0, B_Wq, B_Wk, B_Wv, B_Wo, B_seg_len):

    def _A_ref(x, wqkv, wo):
        B, S, D = x.shape
        H = 32
        Dh = D // H
        qkv = (lambda x, *d: x.transpose(*d))((x @ wqkv).reshape(B, S, 3, H, Dh), 2, 0, 3, 1, 4)
        q, k, v = (qkv[0], qkv[1], qkv[2])
        scale = Dh ** (-0.5)
        scores = jnp.einsum('bhqd,bhkd->bhqk', q, k) * scale
        p = _softmax(scores, axis=-1)
        o = jnp.einsum('bhqk,bhkd->bhqd', p, v)
        return (lambda x, *d: x.transpose(*d))(o, 0, 2, 1, 3).reshape(B, S, D) @ wo

    def _B_ref(x, mem0, Wq, Wk, Wv, Wo, seg_len):
        B, S, Dm = x.shape
        H, Dh = (Wq.shape[1], Wq.shape[2])
        M = mem0.shape[1]
        scale = Dh ** (-0.5)
        n_seg = S // seg_len
        L = M + seg_len
        idx = jnp.arange(L)
        mask = (idx[:, None] < M) | (idx[:, None] >= idx[None, :])
        mem = mem0
        outs = []
        for s in range(n_seg):
            xs = x[:, s * seg_len:(s + 1) * seg_len, :].copy()
            h = jnp.concatenate([mem, xs], axis=1)
            q = jnp.einsum('btd,dhe->bhte', h, Wq)
            k = jnp.einsum('btd,dhe->bhte', h, Wk)
            v = jnp.einsum('btd,dhe->bhte', h, Wv)
            scores = jnp.einsum('bhqe,bhke->bhqk', q, k) * scale
            scores = jnp.where(mask[None, None], scores, -1000000000.0)
            p = _softmax(scores, axis=-1)
            o = jnp.einsum('bhqk,bhke->bhqe', p, v)
            o = jnp.einsum('bhte,hed->btd', o, Wo)
            mem = o[:, :M, :].copy()
            outs.append(o[:, M:, :])
        return jnp.concatenate(outs, axis=1)
    a = _A_ref(A_x, A_wqkv, A_wo)
    b = _B_ref(B_x, B_mem0, B_Wq, B_Wk, B_Wv, B_Wo, B_seg_len)
    return jnp.concatenate([a, b], axis=-1)
```

```python
import math

import jax
import jax.numpy as jnp
import jax.experimental.pallas as pl
import jax.experimental.pallas.tpu as pltpu

_BF = jnp.bfloat16
_F32 = jnp.float32

_SEQ = 2048
_D = 1024
_HA = 32
_DHA = _D // _HA
_NG = _D // 128
_NT = _SEQ // 128
_KB = 128
_LAG = 2
_HB = 32
_DHB = 128
_M = 8
_SEG = 32
_L = _M + _SEG
_NSEG = _SEQ // _SEG
_GB = 8
_TB = 256
_NTB = _SEQ // _TB
_DCH = _D // _NTB

_QSCALE = (_DHA ** -0.5) * math.log2(math.e)
_BSCALE = _DHB ** -0.5


def _kernel(
    xa_hbm, wqkv_hbm, woa_hbm, xb_hbm, mem0_hbm, wq_hbm, wk_hbm, wv_hbm, wob_hbm,
    out_hbm,
    xa, wqkv, woa, xb, mem0, wq, wk, wv, wob, raw,
    kk, qt, vt, ot, s_scr, m_scr, outa, outb,
    q_scr, k_scr, v_scr, p_scr, o_scr,
    sem_in, sem_raw, sem_wob, sem_outa, sem_outb,
):
  cp_xa = pltpu.make_async_copy(xa_hbm, xa, sem_in.at[0])
  cp_wqkv = pltpu.make_async_copy(wqkv_hbm, wqkv, sem_in.at[1])
  cp_xb = pltpu.make_async_copy(xb_hbm, xb, sem_in.at[2])
  cp_woa = pltpu.make_async_copy(woa_hbm, woa, sem_in.at[3])
  cp_mem = pltpu.make_async_copy(mem0_hbm, mem0, sem_in.at[4])
  cp_wob = [
      pltpu.make_async_copy(
          wob_hbm.at[:, pl.ds(n * 128, 128)], wob.at[n], sem_wob.at[n])
      for n in range(_D // 128)
  ]
  wb_hbm = (wq_hbm, wk_hbm, wv_hbm)
  wb = (wq, wk, wv)

  def raw_copy(i, slot, t):
    return pltpu.make_async_copy(
        wb_hbm[t].at[pl.ds(pl.multiple_of(i * _DCH, _DCH), _DCH)],
        raw.at[slot, t], sem_raw.at[slot, t])

  cp_wqkv.start()
  cp_xa.start()
  for t in range(3):
    raw_copy(0, 0, t).start()
  cp_wqkv.wait()
  cp_xa.wait()
  cp_mem.start()
  cp_xb.start()
  for c in cp_wob:
    c.start()
  cp_woa.start()

  def proj_body(i, carry):
    slot = i % 2

    @pl.when(i + 1 < _NTB)
    def _():
      for t in range(3):
        raw_copy(i + 1, 1 - slot, t).start()

    t0 = pl.multiple_of(i * _TB, _TB)
    x = xa[pl.ds(t0, _TB), :]
    kf = jnp.dot(x, wqkv[:, _D:2 * _D], preferred_element_type=_F32).astype(_BF)
    for g in range(_NG):
      kk[g, pl.ds(t0, _TB), :] = kf[:, g * 128:(g + 1) * 128]
    qf = jnp.dot(x, wqkv[:, 0:_D], preferred_element_type=_F32) * _QSCALE
    qf = qf.astype(_BF).T
    vf = jnp.dot(x, wqkv[:, 2 * _D:3 * _D], preferred_element_type=_F32)
    vf = vf.astype(_BF).T
    for g in range(_NG):
      for u in range(_TB // 128):
        qt[g, i * (_TB // 128) + u] = qf[g * 128:(g + 1) * 128, u * 128:(u + 1) * 128]
        vt[g, i * (_TB // 128) + u] = vf[g * 128:(g + 1) * 128, u * 128:(u + 1) * 128]
    d0 = pl.multiple_of(i * _DCH, _DCH)
    for t in range(3):
      raw_copy(i, slot, t).wait()
      wb[t][:, pl.ds(d0, _DCH), :] = jnp.swapaxes(raw[slot, t], 0, 1)
    return carry

  jax.lax.fori_loop(0, _NTB, proj_body, 0)

  nc = _SEQ // _KB

  def q_stationary(g, q, j):
    parts = [
        qt[g, q, 32 * j:32 * j + 32, :] if t == j else jnp.zeros((32, 128), _BF)
        for t in range(4)
    ]
    return jnp.concatenate(parts, axis=0)

  def pass1_chunk(g, qs, buf, c, m):
    s = jnp.dot(kk[g, c * _KB:(c + 1) * _KB, :], qs, preferred_element_type=_F32)
    s_scr[buf, c * _KB:(c + 1) * _KB, :] = s
    mm = s.reshape(_KB // 8, 8, 128).max(axis=0)
    return mm if m is None else jnp.maximum(m, mm)

  def pass2_chunk(g, j, buf, c, m, l, acc):
    s = s_scr[buf, c * _KB:(c + 1) * _KB, :]
    p3 = jnp.exp2(s.reshape(_KB // 8, 8, 128) - m[None])
    ls = p3.sum(axis=0)
    p = p3.reshape(_KB, 128).astype(_BF)
    if _KB == 128:
      v = vt[g, c, 32 * j:32 * j + 32, :]
    else:
      v = jnp.concatenate(
          [vt[g, c * (_KB // 128) + u, 32 * j:32 * j + 32, :]
           for u in range(_KB // 128)], axis=1)
    pv = jnp.dot(v, p, preferred_element_type=_F32)
    return (ls if l is None else l + ls), (pv if acc is None else acc + pv)

  def col_max(m):
    return jnp.broadcast_to(jnp.max(m, axis=0, keepdims=True), (8, 128))

  for j in range(_LAG):
    qs = q_stationary(0, 0, j)
    m = None
    for c in range(nc):
      m = pass1_chunk(0, qs, j, c, m)
    m_scr[j] = col_max(m)

  nit = _NG * _NT

  def attn_body(it, carry):
    g, q = it // _NT, it % _NT
    itn = jnp.minimum(it + 1, nit - 1)
    gn, qn = itn // _NT, itn % _NT
    for j in range(4):
      jn = (j + _LAG) % 4
      g1, q1 = (g, q) if j + _LAG < 4 else (gn, qn)
      qs = q_stationary(g1, q1, jn)
      mcur = m_scr[j]
      mn = l = acc = None
      for c in range(nc):
        mn = pass1_chunk(g1, qs, jn, c, mn)
        l, acc = pass2_chunk(g, j, j, c, mcur, l, acc)
      lt = jnp.sum(l, axis=0, keepdims=True)
      ot[g, q, 32 * j:32 * j + 32, :] = (acc * (1.0 / lt)).astype(_BF)
      m_scr[jn] = col_max(mn)
    return carry

  jax.lax.fori_loop(0, nit, attn_body, 0)

  cp_woa.wait()

  def outa_copy(i):
    t0 = pl.multiple_of(i * _TB, _TB)
    return pltpu.make_async_copy(
        outa.at[pl.ds(t0, _TB), :], out_hbm.at[pl.ds(t0, _TB), pl.ds(0, _D)], sem_outa)

  def outp_body(i, carry):
    rows = []
    for u in range(_TB // 128):
      o = jnp.concatenate(
          [ot[g, i * (_TB // 128) + u].T for g in range(_NG)], axis=1)
      rows.append(o)
    o = jnp.concatenate(rows, axis=0)
    t0 = pl.multiple_of(i * _TB, _TB)
    outa[pl.ds(t0, _TB), :] = jnp.dot(
        o, woa[...], preferred_element_type=_F32).astype(_BF)
    outa_copy(i).start()
    return carry

  jax.lax.fori_loop(0, _NTB, outp_body, 0)

  cp_mem.wait()
  cp_xb.wait()
  for c in cp_wob:
    c.wait()

  row = jax.lax.broadcasted_iota(jnp.int32, (_L, _L), 0)
  col = jax.lax.broadcasted_iota(jnp.int32, (_L, _L), 1)
  mask = (row < _M) | (row >= col)

  def outb_copy(s):
    r0 = pl.multiple_of(s * _SEG, _SEG)
    return pltpu.make_async_copy(
        outb.at[pl.ds(r0, _SEG), :], out_hbm.at[pl.ds(r0, _SEG), pl.ds(_D, _D)], sem_outb)

  def step(s, mem):
    r0 = pl.multiple_of(s * _SEG, _SEG)
    xs = xb[pl.ds(r0, _SEG), :].astype(_F32)
    h = jnp.concatenate([mem, xs], axis=0)

    def proj(hd):
      q_scr[hd] = jnp.dot(h, wq[hd], preferred_element_type=_F32).astype(_BF)
      k_scr[hd] = jnp.dot(h, wk[hd], preferred_element_type=_F32).astype(_BF)
      v_scr[hd] = jnp.dot(h, wv[hd], preferred_element_type=_F32).astype(_BF)

    def scores(hd):
      sc = jax.lax.dot_general(
          q_scr[hd], k_scr[hd], (((1,), (1,)), ((), ())),
          preferred_element_type=_F32) * _BSCALE
      sc = jnp.where(mask, sc, -1e9)
      m = jnp.max(sc, axis=-1, keepdims=True)
      p = jnp.exp(sc - m)
      l = jnp.sum(p, axis=-1, keepdims=True)
      p_scr[hd] = (p * (1.0 / l)).astype(_BF)

    def pv(hd):
      o = jnp.dot(p_scr[hd], v_scr[hd], preferred_element_type=_F32)
      o_scr[:, hd * _DHB:(hd + 1) * _DHB] = o.astype(_BF).astype(_F32)

    ng = _HB // _GB
    for t in range(ng + 2):
      if t < ng:
        for hd in range(t * _GB, (t + 1) * _GB):
          proj(hd)
      if 0 <= t - 1 < ng:
        for hd in range((t - 1) * _GB, t * _GB):
          scores(hd)
      if 0 <= t - 2 < ng:
        for hd in range((t - 2) * _GB, (t - 1) * _GB):
          pv(hd)
    oa = o_scr[...]
    out = jnp.concatenate(
        [jnp.dot(oa, wob[n], preferred_element_type=_F32) for n in range(_D // 128)],
        axis=1)
    outb[pl.ds(r0, _SEG), :] = out[_M:].astype(_BF)
    outb_copy(s).start()
    return out[:_M].astype(_BF).astype(_F32)

  jax.lax.fori_loop(0, _NSEG, step, mem0[...].astype(_F32))

  def wait_a(i, carry):
    outa_copy(i).wait()
    return carry

  jax.lax.fori_loop(0, _NTB, wait_a, 0)

  def wait_b(s, carry):
    outb_copy(s).wait()
    return carry

  jax.lax.fori_loop(0, _NSEG, wait_b, 0)


@jax.jit
def pallas_concat_heads__softmax_full_mha__memory_aug_recurrent_mem_tr__prompt_kernel(
    A_x: jax.Array,
    A_wqkv: jax.Array,
    A_wo: jax.Array,
    B_x: jax.Array,
    B_mem0: jax.Array,
    B_Wq: jax.Array,
    B_Wk: jax.Array,
    B_Wv: jax.Array,
    B_Wo: jax.Array,
    B_seg_len=_SEG,
):
  del B_seg_len
  vmem = pltpu.VMEM
  scratch = [
      vmem((_SEQ, _D), _BF),
      vmem((_D, 3 * _D), _BF),
      vmem((_D, _D), _BF),
      vmem((_SEQ, _D), _BF),
      vmem((_M, _D), _BF),
      vmem((_HB, _D, _DHB), _BF),
      vmem((_HB, _D, _DHB), _BF),
      vmem((_HB, _D, _DHB), _BF),
      vmem((_D // 128, _HB * _DHB, 128), _BF),
      vmem((2, 3, _DCH, _HB, _DHB), _BF),
      vmem((_NG, _SEQ, 128), _BF),
      vmem((_NG, _NT, 128, 128), _BF),
      vmem((_NG, _NT, 128, 128), _BF),
      vmem((_NG, _NT, 128, 128), _BF),
      vmem((4, _SEQ, 128), _F32),
      vmem((4, 8, 128), _F32),
      vmem((_SEQ, _D), _BF),
      vmem((_SEQ, _D), _BF),
      vmem((_HB, _L, _DHB), _BF),
      vmem((_HB, _L, _DHB), _BF),
      vmem((_HB, _L, _DHB), _BF),
      vmem((_HB, _L, _L), _BF),
      vmem((_L, _HB * _DHB), _F32),
      pltpu.SemaphoreType.DMA((5,)),
      pltpu.SemaphoreType.DMA((2, 3)),
      pltpu.SemaphoreType.DMA((_D // 128,)),
      pltpu.SemaphoreType.DMA(()),
      pltpu.SemaphoreType.DMA(()),
  ]
  any_spec = pl.BlockSpec(memory_space=pl.ANY)
  out = pl.pallas_call(
      _kernel,
      out_shape=jax.ShapeDtypeStruct((_SEQ, 2 * _D), _BF),
      in_specs=[any_spec] * 9,
      out_specs=any_spec,
      scratch_shapes=scratch,
      compiler_params=pltpu.CompilerParams(vmem_limit_bytes=112 * 1024 * 1024),
      name="fused_mha_rmt",
  )(
      A_x.reshape(_SEQ, _D),
      A_wqkv,
      A_wo,
      B_x.reshape(_SEQ, _D),
      B_mem0.reshape(_M, _D),
      B_Wq,
      B_Wk,
      B_Wv,
      B_Wo.reshape(_HB * _DHB, _D),
  )
  return out.reshape(1, _SEQ, 2 * _D)
```

```python
import math

import numpy as np

import jax
import jax.numpy as jnp
import jax.experimental.pallas as pl
import jax.experimental.pallas.tpu as pltpu

_BF = jnp.bfloat16
_F32 = jnp.float32

_SEQ = 2048
_D = 1024
_HA = 32
_DHA = _D // _HA
_NG = _D // 128
_NT = _SEQ // 128
_KB = 128
_LAG = 2
_SKEW = 1
_HB = 32
_DHB = 128
_M = 8
_SEG = 32
_L = _M + _SEG
_NSEG = _SEQ // _SEG
_GB = 8
_UNR = 2
_TB = 256
_NTB = _SEQ // _TB
_PN = 256
_RD = 64

_QSCALE = (_DHA ** -0.5) * math.log2(math.e)
_BSCALE = _DHB ** -0.5
_HI_MASK = np.uint32(0xFFFF0000)


def _interleave(streams):
  gens = [s[0] for s in streams]
  totals = [float(s[1]) for s in streams]
  prog = [0.0] * len(gens)
  alive = [True] * len(gens)
  while any(alive):
    i = min((k for k in range(len(gens)) if alive[k]),
            key=lambda k: prog[k] / totals[k])
    try:
      prog[i] += next(gens[i])
    except StopIteration:
      alive[i] = False


def _kernel(
    xa_hbm, wqkv_hbm, woa_hbm, xb_hbm, mem0_hbm, wq_hbm, wk_hbm, wv_hbm, wob_hbm,
    out_hbm,
    xa, wqkv, woa, xb, mem0, wq, wk, wv, wob, raw,
    kk, qt, vt, ot, s_scr, m_scr, outa, outb,
    q_scr, k_scr, v_scr, p_scr, o_scr,
    sem_in, sem_x, sem_raw, sem_wob, sem_outa, sem_outb,
):
  def xa_copy(i):
    t0 = pl.multiple_of(i * _TB, _TB)
    return pltpu.make_async_copy(
        xa_hbm.at[pl.ds(t0, _TB)], xa.at[pl.ds(t0, _TB)], sem_x.at[i])

  cp_w = [
      pltpu.make_async_copy(
          wqkv_hbm.at[:, pl.ds(p * _D, _D)], wqkv.at[:, pl.ds(p * _D, _D)], sem_in.at[p])
      for p in range(3)
  ]
  cp_xb = pltpu.make_async_copy(xb_hbm, xb, sem_in.at[3])
  cp_woa = pltpu.make_async_copy(woa_hbm, woa, sem_in.at[4])
  cp_mem = pltpu.make_async_copy(mem0_hbm, mem0, sem_in.at[5])

  def wob_copy(n):
    n0 = n * 128 if isinstance(n, int) else pl.multiple_of(n * 128, 128)
    return pltpu.make_async_copy(
        wob_hbm.at[:, pl.ds(n0, 128)], wob.at[n], sem_wob.at[n])

  wb = (wq, wk, wv)
  wb_u32 = tuple(w.bitcast(jnp.uint32) for w in (wq_hbm, wk_hbm, wv_hbm))

  def raw_copy(i, slot, t, c):
    return pltpu.make_async_copy(
        wb_u32[t].at[:, 2 * i + c, :], raw.at[slot, t, c], sem_raw.at[slot, t, c])

  def raw_start(i, slot):
    for t in range(3):
      for c in range(2):
        raw_copy(i, slot, t, c).start()

  def raw_wait(slot):
    for t in range(3):
      for c in range(2):
        raw_copy(0, slot, t, c).wait()

  def proj_stream(i, first=False):
    t0 = pl.multiple_of(i * _TB, _TB)
    x = xa[pl.ds(t0, _TB), :]
    for part in (1, 0, 2):
      if first:
        cp_w[part].wait()
        if part == 0:
          cp_w[2].start()
        if part == 2:
          xa_copy(1).start()
          raw_start(0, 0)
          cp_mem.start()
      for pn in range(_D // _PN):
        c0 = part * _D + pn * _PN
        y = jnp.dot(x, wqkv[:, c0:c0 + _PN], preferred_element_type=_F32)
        if part == 0:
          y = y * _QSCALE
        y = y.astype(_BF)
        for gg in range(_PN // 128):
          g = pn * (_PN // 128) + gg
          if part == 1:
            kk[g, pl.ds(t0, _TB), :] = y[:, gg * 128:(gg + 1) * 128]
          else:
            dst = qt if part == 0 else vt
            for u in range(_TB // 128):
              dst[g, i * (_TB // 128) + u] = (
                  y[u * 128:(u + 1) * 128, gg * 128:(gg + 1) * 128].T)
        yield 1.0
  proj_total = 3 * (_D // _PN)

  def relayout_stream(i, slot):
    for t in range(3):
      for c in range(2):
        for d in range(0, _D, _RD):
          w = raw[slot, t, c, d:d + _RD, :]
          lo = pltpu.bitcast(w << 16, _F32).astype(_BF)
          hi = pltpu.bitcast(w & _HI_MASK, _F32).astype(_BF)
          wb[t][4 * i + 2 * c, d:d + _RD, :] = lo
          wb[t][4 * i + 2 * c + 1, d:d + _RD, :] = hi
          yield 1.0
  relayout_total = 3 * 2 * (_D // _RD)

  cp_w[1].start()
  xa_copy(0).start()
  cp_w[0].start()
  xa_copy(0).wait()
  for _ in proj_stream(0, first=True):
    pass

  def proj_body(i, carry):
    slot = i % 2
    raw_start(i, slot)

    @pl.when(i + 1 < _NTB)
    def _():
      xa_copy(i + 1).start()

    wob_copy(i - 1).start()

    @pl.when(i == 5)
    def _():
      cp_xb.start()

    xa_copy(i).wait()
    raw_wait(1 - slot)
    _interleave([(proj_stream(i), proj_total),
                 (relayout_stream(i - 1, 1 - slot), relayout_total)])
    return carry

  jax.lax.fori_loop(1, _NTB, proj_body, 0)
  wob_copy(_NTB - 1).start()
  cp_woa.start()

  nc = _SEQ // _KB
  nit = _NG * _NT

  def q_stationary(g, q, j):
    parts = [
        qt[g, q, 32 * j:32 * j + 32, :] if t == j else jnp.zeros((32, 128), _BF)
        for t in range(4)
    ]
    return jnp.concatenate(parts, axis=0)

  def pass1_chunk(g, qs, buf, c, m):
    s = jnp.dot(kk[g, c * _KB:(c + 1) * _KB, :], qs, preferred_element_type=_F32)
    s_scr[buf, c * _KB:(c + 1) * _KB, :] = s
    mm = s.reshape(_KB // 8, 8, 128).max(axis=0)
    return mm if m is None else jnp.maximum(m, mm)

  def pass2_chunk(g, j, buf, c, m, l, acc):
    s = s_scr[buf, c * _KB:(c + 1) * _KB, :]
    p3 = jnp.exp2(s.reshape(_KB // 8, 8, 128) - m[None])
    ls = p3.sum(axis=0)
    p = p3.reshape(_KB, 128).astype(_BF)
    v = vt[g, c, 32 * j:32 * j + 32, :]
    pv = jnp.dot(v, p, preferred_element_type=_F32)
    return (ls if l is None else l + ls), (pv if acc is None else acc + pv)

  def col_max(m):
    return jnp.broadcast_to(jnp.max(m, axis=0, keepdims=True), (8, 128))

  def a_prologue():
    for j in range(_LAG):
      qs = q_stationary(0, 0, j)
      m = None
      for c in range(nc):
        m = pass1_chunk(0, qs, j, c, m)
        yield 1.0
      m_scr[j] = col_max(m)

  raw_wait((_NTB - 1) % 2)
  _interleave([(a_prologue(), _LAG * nc),
               (relayout_stream(_NTB - 1, (_NTB - 1) % 2), relayout_total)])

  def a_stream(it0, n_it):
    for ii in range(n_it):
      it = it0 + ii
      g, q = it // _NT, it % _NT
      itn = jnp.minimum(it + 1, nit - 1)
      gn, qn = itn // _NT, itn % _NT
      for j in range(4):
        jn = (j + _LAG) % 4
        g1, q1 = (g, q) if j + _LAG < 4 else (gn, qn)
        qs = q_stationary(g1, q1, jn)
        mcur = m_scr[j]
        mn = l = acc = None
        c1 = c2 = 0
        for t in range(nc + _SKEW):
          if c2 < nc:
            l, acc = pass2_chunk(g, j, j, c2, mcur, l, acc)
            c2 += 1
            yield _KB / 16.0
            if c2 == nc:
              lt = jnp.sum(l, axis=0, keepdims=True)
              ot[g, q, 32 * j:32 * j + 32, :] = (acc * (1.0 / lt)).astype(_BF)
          if t >= _SKEW and c1 < nc:
            mn = pass1_chunk(g1, qs, jn, c1, mn)
            c1 += 1
            yield _KB / 4.0
        m_scr[jn] = col_max(mn)

  def a_total(n_it):
    return n_it * 4 * nc * (_KB / 4.0 + _KB / 16.0)

  cp_mem.wait()
  cp_xb.wait()
  for n in range(_D // 128):
    wob_copy(n).wait()

  row = jax.lax.broadcasted_iota(jnp.int32, (_L, _L), 0)
  col = jax.lax.broadcasted_iota(jnp.int32, (_L, _L), 1)
  mask = (row < _M) | (row >= col)

  def outb_copy(s):
    r0 = pl.multiple_of(s * _SEG, _SEG)
    return pltpu.make_async_copy(
        outb.at[pl.ds(r0, _SEG), :], out_hbm.at[pl.ds(r0, _SEG), pl.ds(_D, _D)], sem_outb)

  def b_stream(s, mem, result):
    r0 = pl.multiple_of(s * _SEG, _SEG)
    xs = xb[pl.ds(r0, _SEG), :].astype(_F32)
    h = jnp.concatenate([mem, xs], axis=0)

    def proj(hd):
      q = jnp.dot(h, wq[hd], preferred_element_type=_F32).astype(_BF)
      q_scr[hd] = q.astype(_F32)
      yield 80.0
      k_scr[hd] = jnp.dot(h, wk[hd], preferred_element_type=_F32).astype(_BF)
      yield 80.0
      v_scr[hd] = jnp.dot(h, wv[hd], preferred_element_type=_F32).astype(_BF)
      yield 80.0

    def scores(hd):
      sc = jax.lax.dot_general(
          q_scr[hd], k_scr[hd], (((1,), (1,)), ((), ())),
          preferred_element_type=_F32) * _BSCALE
      sc = jnp.where(mask, sc, -1e9)
      m = jnp.max(sc, axis=-1, keepdims=True)
      p = jnp.exp(sc - m)
      l = jnp.sum(p, axis=-1, keepdims=True)
      p_scr[hd] = (p * (1.0 / l)).astype(_BF).astype(_F32)
      yield 12.0

    def pv(hd):
      o = jnp.dot(p_scr[hd], v_scr[hd], preferred_element_type=_F32)
      o_scr[:, hd * _DHB:(hd + 1) * _DHB] = o.astype(_BF).astype(_F32)
      yield 12.0

    accs = [None] * (_D // 128)

    def wo_part(gi):
      sl = slice(gi * _GB * _DHB, (gi + 1) * _GB * _DHB)
      for n in range(_D // 128):
        d = jnp.dot(o_scr[:, sl], wob[n, sl, :], preferred_element_type=_F32)
        accs[n] = d if accs[n] is None else accs[n] + d
        yield 10.0 * _GB

    ng = _HB // _GB
    for t in range(ng + 3):
      if t < ng:
        for hd in range(t * _GB, (t + 1) * _GB):
          yield from proj(hd)
      if 0 <= t - 1 < ng:
        for hd in range((t - 1) * _GB, t * _GB):
          yield from scores(hd)
      if 0 <= t - 2 < ng:
        for hd in range((t - 2) * _GB, (t - 1) * _GB):
          yield from pv(hd)
      if 0 <= t - 3 < ng:
        yield from wo_part(t - 3)
    out = jnp.concatenate(accs, axis=1)
    outb[pl.ds(r0, _SEG), :] = out[_M:].astype(_BF)
    outb_copy(s).start()
    result.append(out[:_M].astype(_BF).astype(_F32))
  b_total = _HB * (240.0 + 24.0) + 2560.0

  def b_multi(s0, mem, result):
    for u in range(_UNR):
      r = []
      yield from b_stream(s0 + u, mem, r)
      mem = r[0]
    result.append(mem)

  def main_body(i, mem):
    result = []
    _interleave([(b_multi(i * _UNR, mem, result), _UNR * b_total),
                 (a_stream(2 * _UNR * i, 2 * _UNR), a_total(2 * _UNR))])
    return result[0]

  jax.lax.fori_loop(0, _NSEG // _UNR, main_body, mem0[...].astype(_F32))

  cp_woa.wait()

  def outa_copy(i):
    t0 = pl.multiple_of(i * _TB, _TB)
    return pltpu.make_async_copy(
        outa.at[pl.ds(t0, _TB), :], out_hbm.at[pl.ds(t0, _TB), pl.ds(0, _D)], sem_outa)

  def outp_body(i, carry):
    rows = []
    for u in range(_TB // 128):
      rows.append(jnp.concatenate(
          [ot[g, i * (_TB // 128) + u].T for g in range(_NG)], axis=1))
    o = jnp.concatenate(rows, axis=0)
    t0 = pl.multiple_of(i * _TB, _TB)
    outa[pl.ds(t0, _TB), :] = jnp.dot(
        o, woa[...], preferred_element_type=_F32).astype(_BF)
    outa_copy(i).start()
    return carry

  jax.lax.fori_loop(0, _NTB, outp_body, 0)

  def wait_a(i, carry):
    outa_copy(i).wait()
    return carry

  jax.lax.fori_loop(0, _NTB, wait_a, 0)

  def wait_b(s, carry):
    outb_copy(s).wait()
    return carry

  jax.lax.fori_loop(0, _NSEG, wait_b, 0)


@jax.jit
def pallas_concat_heads__softmax_full_mha__memory_aug_recurrent_mem_tr__prompt_kernel(
    A_x: jax.Array,
    A_wqkv: jax.Array,
    A_wo: jax.Array,
    B_x: jax.Array,
    B_mem0: jax.Array,
    B_Wq: jax.Array,
    B_Wk: jax.Array,
    B_Wv: jax.Array,
    B_Wo: jax.Array,
    B_seg_len=_SEG,
):
  del B_seg_len
  vmem = pltpu.VMEM
  dma = pltpu.SemaphoreType.DMA
  scratch = [
      vmem((_SEQ, _D), _BF),
      vmem((_D, 3 * _D), _BF),
      vmem((_D, _D), _BF),
      vmem((_SEQ, _D), _BF),
      vmem((_M, _D), _BF),
      vmem((_HB, _D, _DHB), _BF),
      vmem((_HB, _D, _DHB), _BF),
      vmem((_HB, _D, _DHB), _BF),
      vmem((_D // 128, _HB * _DHB, 128), _BF),
      vmem((2, 3, 2, _D, 128), jnp.uint32),
      vmem((_NG, _SEQ, 128), _BF),
      vmem((_NG, _NT, 128, 128), _BF),
      vmem((_NG, _NT, 128, 128), _BF),
      vmem((_NG, _NT, 128, 128), _BF),
      vmem((4, _SEQ, 128), _F32),
      vmem((4, 8, 128), _F32),
      vmem((_SEQ, _D), _BF),
      vmem((_SEQ, _D), _BF),
      vmem((_HB, _L, _DHB), _F32),
      vmem((_HB, _L, _DHB), _BF),
      vmem((_HB, _L, _DHB), _BF),
      vmem((_HB, _L, _L), _F32),
      vmem((_L, _HB * _DHB), _F32),
      dma((6,)),
      dma((_NTB,)),
      dma((2, 3, 2)),
      dma((_D // 128,)),
      dma(()),
      dma(()),
  ]
  any_spec = pl.BlockSpec(memory_space=pl.ANY)
  out = pl.pallas_call(
      _kernel,
      out_shape=jax.ShapeDtypeStruct((_SEQ, 2 * _D), _BF),
      in_specs=[any_spec] * 9,
      out_specs=any_spec,
      scratch_shapes=scratch,
      compiler_params=pltpu.CompilerParams(vmem_limit_bytes=112 * 1024 * 1024),
      name="fused_mha_rmt",
  )(
      A_x.reshape(_SEQ, _D),
      A_wqkv,
      A_wo,
      B_x.reshape(_SEQ, _D),
      B_mem0.reshape(_M, _D),
      B_Wq,
      B_Wk,
      B_Wv,
      B_Wo.reshape(_HB * _DHB, _D),
  )
  return out.reshape(1, _SEQ, 2 * _D)
```

```python
import math

import numpy as np

import jax
import jax.numpy as jnp
import jax.experimental.pallas as pl
import jax.experimental.pallas.tpu as pltpu

_BF = jnp.bfloat16
_F32 = jnp.float32

_SEQ = 2048
_D = 1024
_HA = 32
_DHA = _D // _HA
_NG = _D // 128
_NT = _SEQ // 128
_KB = 128
_LAG = 2
_SKEW = 1
_HB = 32
_DHB = 128
_M = 8
_SEG = 32
_L = _M + _SEG
_NSEG = _SEQ // _SEG
_GB = 8
_UNR = 2
_TB = 256
_NTB = _SEQ // _TB
_PN = 256
_RD = 64

_QSCALE = (_DHA ** -0.5) * math.log2(math.e)
_BSCALE = _DHB ** -0.5
_LOG2E = math.log2(math.e)
_HI_MASK = np.uint32(0xFFFF0000)


def _interleave(streams):
  gens = [s[0] for s in streams]
  totals = [float(s[1]) for s in streams]
  prog = [0.0] * len(gens)
  alive = [True] * len(gens)
  while any(alive):
    i = min((k for k in range(len(gens)) if alive[k]),
            key=lambda k: prog[k] / totals[k])
    try:
      prog[i] += next(gens[i])
    except StopIteration:
      alive[i] = False


def _kernel(
    xa_hbm, wqkv_hbm, woa_hbm, xb_hbm, mem0_hbm, wq_hbm, wk_hbm, wv_hbm, wob_hbm,
    out_hbm,
    xa, wqkv, woa, xb, mem0, wq, wk, wv, wob, raw,
    kk, qt, vt, ot, s_scr, m_scr, outa, outb,
    q_scr, k_scr, v_scr, p_scr, o_scr,
    sem_in, sem_x, sem_xb, sem_raw, sem_wob, sem_outa, sem_outb,
):
  def xa_copy(i):
    t0 = pl.multiple_of(i * _TB, _TB)
    return pltpu.make_async_copy(
        xa_hbm.at[pl.ds(t0, _TB)], xa.at[pl.ds(t0, _TB)], sem_x.at[i])

  cp_w = [
      pltpu.make_async_copy(
          wqkv_hbm.at[:, pl.ds(p * _D, _D)], wqkv.at[:, pl.ds(p * _D, _D)], sem_in.at[p])
      for p in range(3)
  ]

  def xb_copy(i):
    r0 = i * _TB if isinstance(i, int) else pl.multiple_of(i * _TB, _TB)
    return pltpu.make_async_copy(
        xb_hbm.at[pl.ds(r0, _TB)], xb.at[pl.ds(r0, _TB)], sem_xb.at[i])

  cp_woa = pltpu.make_async_copy(woa_hbm, woa, sem_in.at[4])
  cp_mem = pltpu.make_async_copy(mem0_hbm, mem0, sem_in.at[5])

  def wob_copy(n):
    n0 = n * 128 if isinstance(n, int) else pl.multiple_of(n * 128, 128)
    return pltpu.make_async_copy(
        wob_hbm.at[:, pl.ds(n0, 128)], wob.at[n], sem_wob.at[n])

  wb = (wq, wk, wv)
  wb_u32 = tuple(w.bitcast(jnp.uint32) for w in (wq_hbm, wk_hbm, wv_hbm))

  def raw_copy(i, slot, t, c):
    return pltpu.make_async_copy(
        wb_u32[t].at[:, 2 * i + c, :], raw.at[slot, t, c], sem_raw.at[slot, t, c])

  def raw_start(i, slot):
    for t in range(3):
      for c in range(2):
        raw_copy(i, slot, t, c).start()

  def raw_wait(slot):
    for t in range(3):
      for c in range(2):
        raw_copy(0, slot, t, c).wait()

  def proj_stream(i, first=False):
    t0 = pl.multiple_of(i * _TB, _TB)
    x = xa[pl.ds(t0, _TB), :]
    for part in (0, 2, 1):
      if first:
        cp_w[part].wait()
        if part == 0:
          cp_w[1].start()
          xa_copy(1).start()
          raw_start(0, 0)
        if part == 2:
          cp_mem.start()
          wob_copy(0).start()
          xb_copy(0).start()
      for pn in range(_D // _PN):
        c0 = part * _D + pn * _PN
        y = jnp.dot(x, wqkv[:, c0:c0 + _PN], preferred_element_type=_F32)
        if part == 0:
          y = y * _QSCALE
        y = y.astype(_BF)
        for gg in range(_PN // 128):
          g = pn * (_PN // 128) + gg
          if part == 1:
            kk[g, pl.ds(t0, _TB), :] = y[:, gg * 128:(gg + 1) * 128]
          else:
            dst = qt if part == 0 else vt
            for u in range(_TB // 128):
              dst[g, i * (_TB // 128) + u] = (
                  y[u * 128:(u + 1) * 128, gg * 128:(gg + 1) * 128].T)
        yield 1.0
  proj_total = 3 * (_D // _PN)

  def relayout_stream(i, slot):
    for t in range(3):
      for c in range(2):
        for d in range(0, _D, _RD):
          w = raw[slot, t, c, d:d + _RD, :]
          lo = pltpu.bitcast(w << 16, _F32).astype(_BF)
          hi = pltpu.bitcast(w & _HI_MASK, _F32).astype(_BF)
          wb[t][4 * i + 2 * c, d:d + _RD, :] = lo
          wb[t][4 * i + 2 * c + 1, d:d + _RD, :] = hi
          yield 1.0
  relayout_total = 3 * 2 * (_D // _RD)

  cp_w[0].start()
  xa_copy(0).start()
  cp_w[2].start()
  xa_copy(0).wait()
  for _ in proj_stream(0, first=True):
    pass

  def proj_body(i, carry):
    slot = i % 2
    raw_start(i, slot)

    @pl.when(i + 1 < _NTB)
    def _():
      xa_copy(i + 1).start()

    wob_copy(i).start()
    xb_copy(i).start()
    xa_copy(i).wait()
    raw_wait(1 - slot)
    _interleave([(proj_stream(i), proj_total),
                 (relayout_stream(i - 1, 1 - slot), relayout_total)])
    return carry

  jax.lax.fori_loop(1, _NTB, proj_body, 0)
  cp_woa.start()

  nc = _SEQ // _KB
  nit = _NG * _NT

  def q_stationary(g, q, j):
    parts = [
        qt[g, q, 32 * j:32 * j + 32, :] if t == j else jnp.zeros((32, 128), _BF)
        for t in range(4)
    ]
    return jnp.concatenate(parts, axis=0)

  def pass1_chunk(g, qs, buf, c, m):
    s = jnp.dot(kk[g, c * _KB:(c + 1) * _KB, :], qs, preferred_element_type=_F32)
    s_scr[buf, c * _KB:(c + 1) * _KB, :] = s
    mm = s.reshape(_KB // 8, 8, 128).max(axis=0)
    return mm if m is None else jnp.maximum(m, mm)

  def pass2_chunk(g, j, buf, c, m, l, acc):
    s = s_scr[buf, c * _KB:(c + 1) * _KB, :]
    p3 = jnp.exp2(s.reshape(_KB // 8, 8, 128) - m[None])
    ls = p3.sum(axis=0)
    p = p3.reshape(_KB, 128).astype(_BF)
    v = vt[g, c, 32 * j:32 * j + 32, :]
    pv = jnp.dot(v, p, preferred_element_type=_F32)
    return (ls if l is None else l + ls), (pv if acc is None else acc + pv)

  def col_max(m):
    return jnp.broadcast_to(jnp.max(m, axis=0, keepdims=True), (8, 128))

  def a_prologue():
    for j in range(_LAG):
      qs = q_stationary(0, 0, j)
      m = None
      for c in range(nc):
        m = pass1_chunk(0, qs, j, c, m)
        yield 1.0
      m_scr[j] = col_max(m)

  raw_wait((_NTB - 1) % 2)
  _interleave([(a_prologue(), _LAG * nc),
               (relayout_stream(_NTB - 1, (_NTB - 1) % 2), relayout_total)])

  def a_stream(it0, n_it):
    for ii in range(n_it):
      it = it0 + ii
      g, q = it // _NT, it % _NT
      itn = jnp.minimum(it + 1, nit - 1)
      gn, qn = itn // _NT, itn % _NT
      for j in range(4):
        jn = (j + _LAG) % 4
        g1, q1 = (g, q) if j + _LAG < 4 else (gn, qn)
        qs = q_stationary(g1, q1, jn)
        mcur = m_scr[j]
        mn = l = acc = None
        c1 = c2 = 0
        for t in range(nc + _SKEW):
          if c2 < nc:
            l, acc = pass2_chunk(g, j, j, c2, mcur, l, acc)
            c2 += 1
            yield _KB / 16.0
            if c2 == nc:
              lt = jnp.sum(l, axis=0, keepdims=True)
              ot[g, q, 32 * j:32 * j + 32, :] = (acc * (1.0 / lt)).astype(_BF)
          if t >= _SKEW and c1 < nc:
            mn = pass1_chunk(g1, qs, jn, c1, mn)
            c1 += 1
            yield _KB / 4.0
        m_scr[jn] = col_max(mn)

  def a_total(n_it):
    return n_it * 4 * nc * (_KB / 4.0 + _KB / 16.0)

  cp_mem.wait()
  for i in range(_NTB):
    xb_copy(i).wait()
  for n in range(_D // 128):
    wob_copy(n).wait()

  row = jax.lax.broadcasted_iota(jnp.int32, (_L, _L), 0)
  col = jax.lax.broadcasted_iota(jnp.int32, (_L, _L), 1)
  mask = (row < _M) | (row >= col)

  def outb_copy(s):
    r0 = pl.multiple_of(s * _SEG, _SEG)
    return pltpu.make_async_copy(
        outb.at[pl.ds(r0, _SEG), :], out_hbm.at[pl.ds(r0, _SEG), pl.ds(_D, _D)], sem_outb)

  def b_stream(s, mem, result):
    r0 = pl.multiple_of(s * _SEG, _SEG)
    xs = xb[pl.ds(r0, _SEG), :].astype(_F32)
    h = jnp.concatenate([mem, xs], axis=0)

    def proj(hd):
      q = jnp.dot(h, wq[hd], preferred_element_type=_F32)
      q_scr[hd] = q
      yield 80.0
      k_scr[hd] = jnp.dot(h, wk[hd], preferred_element_type=_F32).astype(_BF)
      yield 80.0
      v_scr[hd] = jnp.dot(h, wv[hd], preferred_element_type=_F32).astype(_BF)
      yield 80.0

    def scores(hd):
      sc = jax.lax.dot_general(
          q_scr[hd], k_scr[hd], (((1,), (1,)), ((), ())),
          preferred_element_type=_F32) * (_BSCALE * _LOG2E)
      sc = jnp.where(mask, sc, -1e9 * _LOG2E)
      m = jnp.max(sc, axis=-1, keepdims=True)
      p = jnp.exp2(sc - m)
      l = jnp.sum(p, axis=-1, keepdims=True)
      r = pl.reciprocal(l, approx=True)
      r = r * (2.0 - l * r)
      p = p * r
      p_scr[hd] = p
      yield 12.0

    def pv(hd):
      o = jnp.dot(p_scr[hd], v_scr[hd], preferred_element_type=_F32)
      o_scr[:, hd * _DHB:(hd + 1) * _DHB] = o
      yield 12.0

    accs = [None] * (_D // 128)

    def wo_part(gi):
      sl = slice(gi * _GB * _DHB, (gi + 1) * _GB * _DHB)
      for n in range(_D // 128):
        d = jnp.dot(o_scr[:, sl], wob[n, sl, :], preferred_element_type=_F32)
        accs[n] = d if accs[n] is None else accs[n] + d
        yield 10.0 * _GB

    ng = _HB // _GB
    for t in range(ng + 3):
      if t < ng:
        for hd in range(t * _GB, (t + 1) * _GB):
          yield from proj(hd)
      if 0 <= t - 1 < ng:
        for hd in range((t - 1) * _GB, t * _GB):
          yield from scores(hd)
      if 0 <= t - 2 < ng:
        for hd in range((t - 2) * _GB, (t - 1) * _GB):
          yield from pv(hd)
      if 0 <= t - 3 < ng:
        yield from wo_part(t - 3)
    out = jnp.concatenate(accs, axis=1)
    outb[pl.ds(r0, _SEG), :] = out[_M:].astype(_BF)
    outb_copy(s).start()
    result.append(out[:_M])
  b_total = _HB * (240.0 + 24.0) + 2560.0

  def b_multi(s0, mem, result):
    for u in range(_UNR):
      r = []
      yield from b_stream(s0 + u, mem, r)
      mem = r[0]
    result.append(mem)

  def main_body(i, mem):
    result = []
    _interleave([(b_multi(i * _UNR, mem, result), _UNR * b_total),
                 (a_stream(2 * _UNR * i, 2 * _UNR), a_total(2 * _UNR))])
    return result[0]

  jax.lax.fori_loop(0, _NSEG // _UNR, main_body, mem0[...].astype(_F32))

  cp_woa.wait()

  def outa_copy(i):
    t0 = pl.multiple_of(i * _TB, _TB)
    return pltpu.make_async_copy(
        outa.at[pl.ds(t0, _TB), :], out_hbm.at[pl.ds(t0, _TB), pl.ds(0, _D)], sem_outa)

  def outp_body(i, carry):
    rows = []
    for u in range(_TB // 128):
      rows.append(jnp.concatenate(
          [ot[g, i * (_TB // 128) + u].T for g in range(_NG)], axis=1))
    o = jnp.concatenate(rows, axis=0)
    t0 = pl.multiple_of(i * _TB, _TB)
    outa[pl.ds(t0, _TB), :] = jnp.dot(
        o, woa[...], preferred_element_type=_F32).astype(_BF)
    outa_copy(i).start()
    return carry

  jax.lax.fori_loop(0, _NTB, outp_body, 0)

  def wait_a(i, carry):
    outa_copy(i).wait()
    return carry

  jax.lax.fori_loop(0, _NTB, wait_a, 0)

  def wait_b(s, carry):
    outb_copy(s).wait()
    return carry

  jax.lax.fori_loop(0, _NSEG, wait_b, 0)


@jax.jit
def pallas_concat_heads__softmax_full_mha__memory_aug_recurrent_mem_tr__prompt_kernel(
    A_x: jax.Array,
    A_wqkv: jax.Array,
    A_wo: jax.Array,
    B_x: jax.Array,
    B_mem0: jax.Array,
    B_Wq: jax.Array,
    B_Wk: jax.Array,
    B_Wv: jax.Array,
    B_Wo: jax.Array,
    B_seg_len=_SEG,
):
  del B_seg_len
  vmem = pltpu.VMEM
  dma = pltpu.SemaphoreType.DMA
  scratch = [
      vmem((_SEQ, _D), _BF),
      vmem((_D, 3 * _D), _BF),
      vmem((_D, _D), _BF),
      vmem((_SEQ, _D), _BF),
      vmem((_M, _D), _BF),
      vmem((_HB, _D, _DHB), _BF),
      vmem((_HB, _D, _DHB), _BF),
      vmem((_HB, _D, _DHB), _BF),
      vmem((_D // 128, _HB * _DHB, 128), _BF),
      vmem((2, 3, 2, _D, 128), jnp.uint32),
      vmem((_NG, _SEQ, 128), _BF),
      vmem((_NG, _NT, 128, 128), _BF),
      vmem((_NG, _NT, 128, 128), _BF),
      vmem((_NG, _NT, 128, 128), _BF),
      vmem((4, _SEQ, 128), _F32),
      vmem((4, 8, 128), _F32),
      vmem((_SEQ, _D), _BF),
      vmem((_SEQ, _D), _BF),
      vmem((_HB, _L, _DHB), _F32),
      vmem((_HB, _L, _DHB), _BF),
      vmem((_HB, _L, _DHB), _BF),
      vmem((_HB, _L, _L), _F32),
      vmem((_L, _HB * _DHB), _F32),
      dma((6,)),
      dma((_NTB,)),
      dma((_NTB,)),
      dma((2, 3, 2)),
      dma((_D // 128,)),
      dma(()),
      dma(()),
  ]
  any_spec = pl.BlockSpec(memory_space=pl.ANY)
  out = pl.pallas_call(
      _kernel,
      out_shape=jax.ShapeDtypeStruct((_SEQ, 2 * _D), _BF),
      in_specs=[any_spec] * 9,
      out_specs=any_spec,
      scratch_shapes=scratch,
      compiler_params=pltpu.CompilerParams(vmem_limit_bytes=112 * 1024 * 1024),
      name="fused_mha_rmt",
  )(
      A_x.reshape(_SEQ, _D),
      A_wqkv,
      A_wo,
      B_x.reshape(_SEQ, _D),
      B_mem0.reshape(_M, _D),
      B_Wq,
      B_Wk,
      B_Wv,
      B_Wo.reshape(_HB * _DHB, _D),
  )
  return out.reshape(1, _SEQ, 2 * _D)
```

```python
import math

import numpy as np

import jax
import jax.numpy as jnp
import jax.experimental.pallas as pl
import jax.experimental.pallas.tpu as pltpu

_BF = jnp.bfloat16
_F32 = jnp.float32

_SEQ = 2048
_D = 1024
_HA = 32
_DHA = _D // _HA
_NG = _D // 128
_NT = _SEQ // 128
_KB = 128
_LAG = 2
_SKEW = 1
_HB = 32
_DHB = 128
_M = 8
_SEG = 32
_L = _M + _SEG
_NSEG = _SEQ // _SEG
_GB = 8
_UNR = 2
_TB = 256
_NTB = _SEQ // _TB
_PN = 256
_RD = 64

_QSCALE = (_DHA ** -0.5) * math.log2(math.e)
_BSCALE = _DHB ** -0.5
_LOG2E = math.log2(math.e)
_HI_MASK = np.uint32(0xFFFF0000)


def _interleave(streams):
  gens = [s[0] for s in streams]
  prog = [0.0] * len(gens)
  alive = [True] * len(gens)

  def pos(k):
    st = streams[k]
    lo, hi = (st[2], st[3]) if len(st) > 2 else (0.0, 1.0)
    return lo + (hi - lo) * prog[k] / st[1]

  while any(alive):
    i = min((k for k in range(len(gens)) if alive[k]), key=pos)
    try:
      prog[i] += next(gens[i])
    except StopIteration:
      alive[i] = False


def _kernel(
    xa_hbm, wqkv_hbm, woa_hbm, xb_hbm, mem0_hbm, wq_hbm, wk_hbm, wv_hbm, wob_hbm,
    out_hbm,
    xa, wqkv, woa, xb, mem0, wq, wk, wv, wob, raw,
    kk, qt, vt, ot, s_scr, m_scr, outa, outb,
    q_scr, k_scr, v_scr, p_scr, o_scr,
    sem_in, sem_x, sem_xb, sem_raw, sem_wob, sem_outa, sem_outb,
):
  def xa_copy(i):
    t0 = pl.multiple_of(i * _TB, _TB)
    return pltpu.make_async_copy(
        xa_hbm.at[pl.ds(t0, _TB)], xa.at[pl.ds(t0, _TB)], sem_x.at[i])

  cp_w = [
      pltpu.make_async_copy(
          wqkv_hbm.at[:, pl.ds(p * _D, _D)], wqkv.at[:, pl.ds(p * _D, _D)], sem_in.at[p])
      for p in range(3)
  ]

  def xb_copy(i):
    r0 = i * _TB if isinstance(i, int) else pl.multiple_of(i * _TB, _TB)
    return pltpu.make_async_copy(
        xb_hbm.at[pl.ds(r0, _TB)], xb.at[pl.ds(r0, _TB)], sem_xb.at[i])

  cp_woa = pltpu.make_async_copy(woa_hbm, woa, sem_in.at[4])
  cp_mem = pltpu.make_async_copy(mem0_hbm, mem0, sem_in.at[5])

  def wob_copy(n):
    n0 = n * 128 if isinstance(n, int) else pl.multiple_of(n * 128, 128)
    return pltpu.make_async_copy(
        wob_hbm.at[:, pl.ds(n0, 128)], wob.at[n], sem_wob.at[n])

  wb = (wq, wk, wv)
  wb_u32 = tuple(w.bitcast(jnp.uint32) for w in (wq_hbm, wk_hbm, wv_hbm))

  def raw_copy(i, slot, t, c):
    return pltpu.make_async_copy(
        wb_u32[t].at[:, 2 * i + c, :], raw.at[slot, t, c], sem_raw.at[slot, t, c])

  def raw_start(i, slot):
    for t in range(3):
      for c in range(2):
        raw_copy(i, slot, t, c).start()

  def raw_wait(slot):
    for t in range(3):
      for c in range(2):
        raw_copy(0, slot, t, c).wait()

  def proj_stream(i, first=False):
    t0 = pl.multiple_of(i * _TB, _TB)
    x = xa[pl.ds(t0, _TB), :]
    for part in (0, 2, 1):
      if first:
        cp_w[part].wait()
        if part == 0:
          cp_w[1].start()
          xa_copy(1).start()
          raw_start(0, 0)
        if part == 2:
          cp_mem.start()
          wob_copy(0).start()
          xb_copy(0).start()
      for pn in range(_D // _PN):
        c0 = part * _D + pn * _PN
        y = jnp.dot(x, wqkv[:, c0:c0 + _PN], preferred_element_type=_F32)
        if part == 0:
          y = y * _QSCALE
        y = y.astype(_BF)
        for gg in range(_PN // 128):
          g = pn * (_PN // 128) + gg
          if part == 1:
            kk[g, pl.ds(t0, _TB), :] = y[:, gg * 128:(gg + 1) * 128]
          else:
            dst = qt if part == 0 else vt
            for u in range(_TB // 128):
              dst[g, i * (_TB // 128) + u] = (
                  y[u * 128:(u + 1) * 128, gg * 128:(gg + 1) * 128].T)
        yield 1.0
  proj_total = 3 * (_D // _PN)

  def relayout_stream(i, slot):
    for t in range(3):
      for c in range(2):
        for d in range(0, _D, _RD):
          w = raw[slot, t, c, d:d + _RD, :]
          lo = pltpu.bitcast(w << 16, _F32).astype(_BF)
          hi = pltpu.bitcast(w & _HI_MASK, _F32).astype(_BF)
          wb[t][4 * i + 2 * c, d:d + _RD, :] = lo
          wb[t][4 * i + 2 * c + 1, d:d + _RD, :] = hi
          yield 1.0
  relayout_total = 3 * 2 * (_D // _RD)

  cp_w[0].start()
  xa_copy(0).start()
  cp_w[2].start()
  xa_copy(0).wait()
  for _ in proj_stream(0, first=True):
    pass

  def proj_body(i, carry):
    slot = i % 2
    raw_start(i, slot)

    @pl.when(i + 1 < _NTB)
    def _():
      xa_copy(i + 1).start()

    wob_copy(i).start()
    xb_copy(i).start()
    xa_copy(i).wait()
    raw_wait(1 - slot)
    _interleave([(proj_stream(i), proj_total),
                 (relayout_stream(i - 1, 1 - slot), relayout_total)])
    return carry

  jax.lax.fori_loop(1, _NTB, proj_body, 0)
  cp_woa.start()

  nc = _SEQ // _KB
  nit = _NG * _NT

  def q_stationary(g, q, j):
    parts = [
        qt[g, q, 32 * j:32 * j + 32, :] if t == j else jnp.zeros((32, 128), _BF)
        for t in range(4)
    ]
    return jnp.concatenate(parts, axis=0)

  def pass1_chunk(g, qs, buf, c, m):
    s = jnp.dot(kk[g, c * _KB:(c + 1) * _KB, :], qs, preferred_element_type=_F32)
    s_scr[buf, c * _KB:(c + 1) * _KB, :] = s
    mm = s.reshape(_KB // 8, 8, 128).max(axis=0)
    return mm if m is None else jnp.maximum(m, mm)

  def pass2_chunk(g, j, buf, c, m, l, acc):
    s = s_scr[buf, c * _KB:(c + 1) * _KB, :]
    p3 = jnp.exp2(s.reshape(_KB // 8, 8, 128) - m[None])
    ls = p3.sum(axis=0)
    p = p3.reshape(_KB, 128).astype(_BF)
    v = vt[g, c, 32 * j:32 * j + 32, :]
    pv = jnp.dot(v, p, preferred_element_type=_F32)
    return (ls if l is None else l + ls), (pv if acc is None else acc + pv)

  def col_max(m):
    return jnp.broadcast_to(jnp.max(m, axis=0, keepdims=True), (8, 128))

  def a_prologue():
    for j in range(_LAG):
      qs = q_stationary(0, 0, j)
      m = None
      for c in range(nc):
        m = pass1_chunk(0, qs, j, c, m)
        yield 1.0
      m_scr[j] = col_max(m)

  raw_wait((_NTB - 1) % 2)
  _interleave([(a_prologue(), _LAG * nc),
               (relayout_stream(_NTB - 1, (_NTB - 1) % 2), relayout_total)])

  def a_stream(it0, n_it):
    for ii in range(n_it):
      it = it0 + ii
      g, q = it // _NT, it % _NT
      itn = jnp.minimum(it + 1, nit - 1)
      gn, qn = itn // _NT, itn % _NT
      for j in range(4):
        jn = (j + _LAG) % 4
        g1, q1 = (g, q) if j + _LAG < 4 else (gn, qn)
        qs = q_stationary(g1, q1, jn)
        mcur = m_scr[j]
        mn = l = acc = None
        c1 = c2 = 0
        for t in range(nc + _SKEW):
          if c2 < nc:
            l, acc = pass2_chunk(g, j, j, c2, mcur, l, acc)
            c2 += 1
            yield _KB / 16.0
            if c2 == nc:
              lt = jnp.sum(l, axis=0, keepdims=True)
              ot[g, q, 32 * j:32 * j + 32, :] = (acc * (1.0 / lt)).astype(_BF)
          if t >= _SKEW and c1 < nc:
            mn = pass1_chunk(g1, qs, jn, c1, mn)
            c1 += 1
            yield _KB / 4.0
        m_scr[jn] = col_max(mn)

  def a_total(n_it):
    return n_it * 4 * nc * (_KB / 4.0 + _KB / 16.0)

  cp_mem.wait()
  for i in range(_NTB):
    xb_copy(i).wait()
  for n in range(_D // 128):
    wob_copy(n).wait()

  row = jax.lax.broadcasted_iota(jnp.int32, (_L, _L), 0)
  col = jax.lax.broadcasted_iota(jnp.int32, (_L, _L), 1)
  mask = (row < _M) | (row >= col)

  n_main = _NSEG // _UNR
  ob_rows = _UNR * _SEG

  def outb_copy(i):
    r0 = pl.multiple_of(i * ob_rows, ob_rows)
    return pltpu.make_async_copy(
        outb.at[pl.ds(r0, ob_rows), :], out_hbm.at[pl.ds(r0, ob_rows), pl.ds(_D, _D)], sem_outb)

  def b_stream(s, mem, result):
    r0 = pl.multiple_of(s * _SEG, _SEG)
    xs = xb[pl.ds(r0, _SEG), :].astype(_F32)
    h = jnp.concatenate([mem, xs], axis=0)

    def proj(hd):
      q = jnp.dot(h, wq[hd], preferred_element_type=_F32)
      q_scr[hd] = q
      yield 80.0
      k_scr[hd] = jnp.dot(h, wk[hd], preferred_element_type=_F32).astype(_BF)
      yield 80.0
      v_scr[hd] = jnp.dot(h, wv[hd], preferred_element_type=_F32).astype(_BF)
      yield 80.0

    def scores(hd):
      sc = jax.lax.dot_general(
          q_scr[hd], k_scr[hd], (((1,), (1,)), ((), ())),
          preferred_element_type=_F32) * (_BSCALE * _LOG2E)
      sc = jnp.where(mask, sc, -1e9 * _LOG2E)
      m = jnp.max(sc, axis=-1, keepdims=True)
      p = jnp.exp2(sc - m)
      l = jnp.sum(p, axis=-1, keepdims=True)
      r = pl.reciprocal(l, approx=True)
      r = r * (2.0 - l * r)
      p = p * r
      p_scr[hd] = p
      yield 12.0

    def pv(hd):
      o = jnp.dot(p_scr[hd], v_scr[hd], preferred_element_type=_F32)
      o_scr[:, hd * _DHB:(hd + 1) * _DHB] = o
      yield 12.0

    accs = [None] * (_D // 128)

    def wo_part(gi):
      sl = slice(gi * _GB * _DHB, (gi + 1) * _GB * _DHB)
      for n in range(_D // 128):
        d = jnp.dot(o_scr[:, sl], wob[n, sl, :], preferred_element_type=_F32)
        accs[n] = d if accs[n] is None else accs[n] + d
        yield 10.0 * _GB

    ng = _HB // _GB
    for t in range(ng + 3):
      if t < ng:
        for hd in range(t * _GB, (t + 1) * _GB):
          yield from proj(hd)
      if 0 <= t - 1 < ng:
        for hd in range((t - 1) * _GB, t * _GB):
          yield from scores(hd)
      if 0 <= t - 2 < ng:
        for hd in range((t - 2) * _GB, (t - 1) * _GB):
          yield from pv(hd)
      if 0 <= t - 3 < ng:
        yield from wo_part(t - 3)
    out = jnp.concatenate(accs, axis=1)
    outb[pl.ds(r0, _SEG), :] = out[_M:].astype(_BF)
    result.append(out[:_M])
  b_total = _HB * (240.0 + 24.0) + 2560.0

  def b_multi(s0, mem, result):
    for u in range(_UNR):
      r = []
      yield from b_stream(s0 + u, mem, r)
      mem = r[0]
    result.append(mem)

  def main_body(i, mem):
    @pl.when(i > 0)
    def _():
      outb_copy(i - 1).start()

    result = []
    t_end = _UNR * (b_total + a_total(2))
    _interleave([(b_multi(i * _UNR, mem, result), _UNR * b_total, 300.0, t_end),
                 (a_stream(2 * _UNR * i, 2 * _UNR), a_total(2 * _UNR), 0.0, t_end)])
    return result[0]

  jax.lax.fori_loop(0, n_main, main_body, mem0[...].astype(_F32))
  outb_copy(n_main - 1).start()

  cp_woa.wait()

  def outa_copy(q):
    t0 = pl.multiple_of(q * 128, 128)
    return pltpu.make_async_copy(
        outa.at[pl.ds(t0, 128), :], out_hbm.at[pl.ds(t0, 128), pl.ds(0, _D)], sem_outa)

  def outp_body(i, carry):
    for u in range(_TB // 128):
      q = i * (_TB // 128) + u
      o = jnp.concatenate([ot[g, q].T for g in range(_NG)], axis=1)
      t0 = pl.multiple_of(q * 128, 128)
      outa[pl.ds(t0, 128), :] = jnp.dot(
          o, woa[...], preferred_element_type=_F32).astype(_BF)
      outa_copy(q).start()
    return carry

  jax.lax.fori_loop(0, _NTB, outp_body, 0)

  def wait_a(i, carry):
    outa_copy(i).wait()
    return carry

  jax.lax.fori_loop(0, _NT, wait_a, 0)

  def wait_b(s, carry):
    outb_copy(s).wait()
    return carry

  jax.lax.fori_loop(0, n_main, wait_b, 0)


@jax.jit
def pallas_concat_heads__softmax_full_mha__memory_aug_recurrent_mem_tr__prompt_kernel(
    A_x: jax.Array,
    A_wqkv: jax.Array,
    A_wo: jax.Array,
    B_x: jax.Array,
    B_mem0: jax.Array,
    B_Wq: jax.Array,
    B_Wk: jax.Array,
    B_Wv: jax.Array,
    B_Wo: jax.Array,
    B_seg_len=_SEG,
):
  del B_seg_len
  vmem = pltpu.VMEM
  dma = pltpu.SemaphoreType.DMA
  scratch = [
      vmem((_SEQ, _D), _BF),
      vmem((_D, 3 * _D), _BF),
      vmem((_D, _D), _BF),
      vmem((_SEQ, _D), _BF),
      vmem((_M, _D), _BF),
      vmem((_HB, _D, _DHB), _BF),
      vmem((_HB, _D, _DHB), _BF),
      vmem((_HB, _D, _DHB), _BF),
      vmem((_D // 128, _HB * _DHB, 128), _BF),
      vmem((2, 3, 2, _D, 128), jnp.uint32),
      vmem((_NG, _SEQ, 128), _BF),
      vmem((_NG, _NT, 128, 128), _BF),
      vmem((_NG, _NT, 128, 128), _BF),
      vmem((_NG, _NT, 128, 128), _BF),
      vmem((4, _SEQ, 128), _F32),
      vmem((4, 8, 128), _F32),
      vmem((_SEQ, _D), _BF),
      vmem((_SEQ, _D), _BF),
      vmem((_HB, _L, _DHB), _F32),
      vmem((_HB, _L, _DHB), _BF),
      vmem((_HB, _L, _DHB), _BF),
      vmem((_HB, _L, _L), _F32),
      vmem((_L, _HB * _DHB), _F32),
      dma((6,)),
      dma((_NTB,)),
      dma((_NTB,)),
      dma((2, 3, 2)),
      dma((_D // 128,)),
      dma(()),
      dma(()),
  ]
  any_spec = pl.BlockSpec(memory_space=pl.ANY)
  out = pl.pallas_call(
      _kernel,
      out_shape=jax.ShapeDtypeStruct((_SEQ, 2 * _D), _BF),
      in_specs=[any_spec] * 9,
      out_specs=any_spec,
      scratch_shapes=scratch,
      compiler_params=pltpu.CompilerParams(vmem_limit_bytes=112 * 1024 * 1024),
      name="fused_mha_rmt",
  )(
      A_x.reshape(_SEQ, _D),
      A_wqkv,
      A_wo,
      B_x.reshape(_SEQ, _D),
      B_mem0.reshape(_M, _D),
      B_Wq,
      B_Wk,
      B_Wv,
      B_Wo.reshape(_HB * _DHB, _D),
  )
  return out.reshape(1, _SEQ, 2 * _D)
```

```python
import math

import numpy as np

import jax
import jax.numpy as jnp
import jax.experimental.pallas as pl
import jax.experimental.pallas.tpu as pltpu

_BF = jnp.bfloat16
_F32 = jnp.float32

_SEQ = 2048
_D = 1024
_HA = 32
_DHA = _D // _HA
_NG = _D // 128
_NT = _SEQ // 128
_KB = 128
_LAG = 2
_SKEW = 1
_HB = 32
_DHB = 128
_M = 8
_SEG = 32
_L = _M + _SEG
_NSEG = _SEQ // _SEG
_GB = 8
_UNR = 2
_TB = 256
_NTB = _SEQ // _TB
_RD = 128
_NP = _D // 128

_QSCALE = (_DHA ** -0.5) * math.log2(math.e)
_BSCALE = _DHB ** -0.5
_LOG2E = math.log2(math.e)
_HI_MASK = np.uint32(0xFFFF0000)


def _interleave(streams):
  gens = [s[0] for s in streams]
  prog = [0.0] * len(gens)
  alive = [True] * len(gens)

  def pos(k):
    st = streams[k]
    lo, hi = (st[2], st[3]) if len(st) > 2 else (0.0, 1.0)
    return lo + (hi - lo) * prog[k] / st[1]

  while any(alive):
    i = min((k for k in range(len(gens)) if alive[k]), key=pos)
    try:
      prog[i] += next(gens[i])
    except StopIteration:
      alive[i] = False


def _kernel(
    xa_hbm, wqkv_hbm, woa_hbm, xb_hbm, mem0_hbm, wq_hbm, wk_hbm, wv_hbm, wob_hbm,
    out_hbm,
    xa, wall, woa, xb, mem0, wob, raw,
    kk, qt, vt, ot, s_scr, m_scr, outa, outb,
    q_scr, k_scr, v_scr, p_scr, o_scr,
    sem_in, sem_x, sem_xb, sem_raw, sem_wob, sem_outa, sem_outb,
):
  def xa_copy(i):
    t0 = pl.multiple_of(i * _TB, _TB)
    return pltpu.make_async_copy(
        xa_hbm.at[pl.ds(t0, _TB)], xa.at[pl.ds(t0, _TB)], sem_x.at[i])

  def wa_copies(p):
    return [
        pltpu.make_async_copy(
            wqkv_hbm.at[:, pl.ds((p * _NP + n) * 128, 128)],
            wall.at[pl.ds((p * _NP + n) * _D, _D), :], sem_in.at[p])
        for n in range(_NP)
    ]

  def wa_start(p):
    for c in wa_copies(p):
      c.start()

  def wa_wait(p):
    for c in wa_copies(p):
      c.wait()

  def wa_panel(n):
    return wall[n * _D:(n + 1) * _D, :]

  def wb_rows(t, hd, r, n):
    start = (3 * _NP + t * _HB + hd) * _D + r
    if isinstance(start, int):
      return pl.ds(start, n)
    return pl.ds(pl.multiple_of(start, _RD), n)

  def xb_copy(i):
    r0 = i * _TB if isinstance(i, int) else pl.multiple_of(i * _TB, _TB)
    return pltpu.make_async_copy(
        xb_hbm.at[pl.ds(r0, _TB)], xb.at[pl.ds(r0, _TB)], sem_xb.at[i])

  cp_woa = pltpu.make_async_copy(woa_hbm, woa, sem_in.at[4])
  cp_mem = pltpu.make_async_copy(mem0_hbm, mem0, sem_in.at[5])

  def wob_copy(n):
    n0 = n * 128 if isinstance(n, int) else pl.multiple_of(n * 128, 128)
    return pltpu.make_async_copy(
        wob_hbm.at[:, pl.ds(n0, 128)], wob.at[n], sem_wob.at[n])

  wb_u32 = tuple(w.bitcast(jnp.uint32) for w in (wq_hbm, wk_hbm, wv_hbm))

  def raw_copy(i, slot, t, c):
    return pltpu.make_async_copy(
        wb_u32[t].at[:, 2 * i + c, :], raw.at[slot, t, c], sem_raw.at[slot, t, c])

  def raw_start(i, slot):
    for t in range(3):
      for c in range(2):
        raw_copy(i, slot, t, c).start()

  def raw_wait(slot):
    for t in range(3):
      for c in range(2):
        raw_copy(0, slot, t, c).wait()

  def proj_stream(i, first=False):
    t0 = pl.multiple_of(i * _TB, _TB)
    x = xa[pl.ds(t0, _TB), :]
    for part in (0, 2, 1):
      if first:
        wa_wait(part)
        if part == 0:
          wa_start(1)
          xa_copy(1).start()
          raw_start(0, 0)
        if part == 2:
          cp_mem.start()
          wob_copy(0).start()
          xb_copy(0).start()
      for g in range(_NP):
        y = jnp.dot(x, wa_panel(part * _NP + g), preferred_element_type=_F32)
        if part == 0:
          y = y * _QSCALE
        y = y.astype(_BF)
        if part == 1:
          kk[g, pl.ds(t0, _TB), :] = y
        else:
          dst = qt if part == 0 else vt
          for u in range(_TB // 128):
            dst[g, i * (_TB // 128) + u] = y[u * 128:(u + 1) * 128, :].T
        yield 1.0
  proj_total = 3 * _NP

  def relayout_stream(i, slot):
    for t in range(3):
      for c in range(2):
        for d in range(0, _D, _RD):
          w = raw[slot, t, c, d:d + _RD, :]
          lo = pltpu.bitcast(w << 16, _F32).astype(_BF)
          hi = pltpu.bitcast(w & _HI_MASK, _F32).astype(_BF)
          wall[wb_rows(t, 4 * i + 2 * c, d, _RD), :] = lo
          wall[wb_rows(t, 4 * i + 2 * c + 1, d, _RD), :] = hi
          yield 1.0
  relayout_total = 3 * 2 * (_D // _RD)

  xa_copy(0).start()
  wa_start(0)
  xa_copy(0).wait()
  wa_start(2)
  for _ in proj_stream(0, first=True):
    pass

  def proj_body(i, carry):
    slot = i % 2
    raw_start(i, slot)

    @pl.when(i + 1 < _NTB)
    def _():
      xa_copy(i + 1).start()

    wob_copy(i).start()
    xb_copy(i).start()
    xa_copy(i).wait()
    raw_wait(1 - slot)
    _interleave([(proj_stream(i), proj_total),
                 (relayout_stream(i - 1, 1 - slot), relayout_total)])
    return carry

  jax.lax.fori_loop(1, _NTB, proj_body, 0)
  cp_woa.start()

  nc = _SEQ // _KB
  nit = _NG * _NT

  def q_stationary(g, q, j):
    parts = [
        qt[g, q, 32 * j:32 * j + 32, :] if t == j else jnp.zeros((32, 128), _BF)
        for t in range(4)
    ]
    return jnp.concatenate(parts, axis=0)

  def pass1_chunk(g, qs, buf, c, m):
    s = jnp.dot(kk[g, c * _KB:(c + 1) * _KB, :], qs, preferred_element_type=_F32)
    s_scr[buf, c * _KB:(c + 1) * _KB, :] = s
    mm = s.reshape(_KB // 8, 8, 128).max(axis=0)
    return mm if m is None else jnp.maximum(m, mm)

  def pass2_chunk(g, j, buf, c, m, l, acc):
    s = s_scr[buf, c * _KB:(c + 1) * _KB, :]
    p3 = jnp.exp2(s.reshape(_KB // 8, 8, 128) - m[None])
    ls = p3.sum(axis=0)
    p = p3.reshape(_KB, 128).astype(_BF)
    v = vt[g, c, 32 * j:32 * j + 32, :]
    pv = jnp.dot(v, p, preferred_element_type=_F32)
    return (ls if l is None else l + ls), (pv if acc is None else acc + pv)

  def col_max(m):
    return jnp.broadcast_to(jnp.max(m, axis=0, keepdims=True), (8, 128))

  def a_prologue():
    for j in range(_LAG):
      qs = q_stationary(0, 0, j)
      m = None
      for c in range(nc):
        m = pass1_chunk(0, qs, j, c, m)
        yield 1.0
      m_scr[j] = col_max(m)

  raw_wait((_NTB - 1) % 2)
  _interleave([(a_prologue(), _LAG * nc),
               (relayout_stream(_NTB - 1, (_NTB - 1) % 2), relayout_total)])

  def a_stream(it0, n_it):
    for ii in range(n_it):
      it = it0 + ii
      g, q = it // _NT, it % _NT
      itn = jnp.minimum(it + 1, nit - 1)
      gn, qn = itn // _NT, itn % _NT
      for j in range(4):
        jn = (j + _LAG) % 4
        g1, q1 = (g, q) if j + _LAG < 4 else (gn, qn)
        qs = q_stationary(g1, q1, jn)
        mcur = m_scr[j]
        mn = l = acc = None
        c1 = c2 = 0
        for t in range(nc + _SKEW):
          if c2 < nc:
            l, acc = pass2_chunk(g, j, j, c2, mcur, l, acc)
            c2 += 1
            yield _KB / 16.0
            if c2 == nc:
              lt = jnp.sum(l, axis=0, keepdims=True)
              ot[g, q, 32 * j:32 * j + 32, :] = (acc * (1.0 / lt)).astype(_BF)
          if t >= _SKEW and c1 < nc:
            mn = pass1_chunk(g1, qs, jn, c1, mn)
            c1 += 1
            yield _KB / 4.0
        m_scr[jn] = col_max(mn)

  def a_total(n_it):
    return n_it * 4 * nc * (_KB / 4.0 + _KB / 16.0)

  cp_mem.wait()
  for i in range(_NTB):
    xb_copy(i).wait()
  for n in range(_D // 128):
    wob_copy(n).wait()

  row = jax.lax.broadcasted_iota(jnp.int32, (_L, _L), 0)
  col = jax.lax.broadcasted_iota(jnp.int32, (_L, _L), 1)
  mask = (row < _M) | (row >= col)

  n_main = _NSEG // _UNR
  ob_rows = _UNR * _SEG

  def outb_copy(i):
    r0 = pl.multiple_of(i * ob_rows, ob_rows)
    return pltpu.make_async_copy(
        outb.at[pl.ds(r0, ob_rows), :], out_hbm.at[pl.ds(r0, ob_rows), pl.ds(_D, _D)], sem_outb)

  def b_stream(s, mem, result):
    r0 = pl.multiple_of(s * _SEG, _SEG)
    xs = xb[pl.ds(r0, _SEG), :].astype(_F32)
    h = jnp.concatenate([mem, xs], axis=0)

    def proj(hd):
      q = jnp.dot(h, wall[wb_rows(0, hd, 0, _D), :], preferred_element_type=_F32)
      q_scr[hd] = q
      yield 80.0
      k_scr[hd] = jnp.dot(h, wall[wb_rows(1, hd, 0, _D), :], preferred_element_type=_F32).astype(_BF)
      yield 80.0
      v_scr[hd] = jnp.dot(h, wall[wb_rows(2, hd, 0, _D), :], preferred_element_type=_F32).astype(_BF)
      yield 80.0

    def scores(hd):
      sc = jax.lax.dot_general(
          q_scr[hd], k_scr[hd], (((1,), (1,)), ((), ())),
          preferred_element_type=_F32) * (_BSCALE * _LOG2E)
      sc = jnp.where(mask, sc, -1e9 * _LOG2E)
      m = jnp.max(sc, axis=-1, keepdims=True)
      p = jnp.exp2(sc - m)
      l = jnp.sum(p, axis=-1, keepdims=True)
      r = pl.reciprocal(l, approx=True)
      r = r * (2.0 - l * r)
      p = p * r
      p_scr[hd] = p
      yield 12.0

    def pv(hd):
      o = jnp.dot(p_scr[hd], v_scr[hd], preferred_element_type=_F32)
      o_scr[:, hd * _DHB:(hd + 1) * _DHB] = o
      yield 12.0

    accs = [None] * (_D // 128)

    def wo_part(gi):
      sl = slice(gi * _GB * _DHB, (gi + 1) * _GB * _DHB)
      for n in range(_D // 128):
        d = jnp.dot(o_scr[:, sl], wob[n, sl, :], preferred_element_type=_F32)
        accs[n] = d if accs[n] is None else accs[n] + d
        yield 10.0 * _GB

    ng = _HB // _GB
    for t in range(ng + 3):
      if t < ng:
        for hd in range(t * _GB, (t + 1) * _GB):
          yield from proj(hd)
      if 0 <= t - 1 < ng:
        for hd in range((t - 1) * _GB, t * _GB):
          yield from scores(hd)
      if 0 <= t - 2 < ng:
        for hd in range((t - 2) * _GB, (t - 1) * _GB):
          yield from pv(hd)
      if 0 <= t - 3 < ng:
        yield from wo_part(t - 3)
    out = jnp.concatenate(accs, axis=1)
    outb[pl.ds(r0, _SEG), :] = out[_M:].astype(_BF)
    result.append(out[:_M])
  b_total = _HB * (240.0 + 24.0) + 2560.0

  def b_multi(s0, mem, result):
    for u in range(_UNR):
      r = []
      yield from b_stream(s0 + u, mem, r)
      mem = r[0]
    result.append(mem)

  def main_body(i, mem):
    @pl.when(i > 0)
    def _():
      outb_copy(i - 1).start()

    result = []
    t_end = _UNR * (b_total + a_total(2))
    _interleave([(b_multi(i * _UNR, mem, result), _UNR * b_total, 300.0, t_end),
                 (a_stream(2 * _UNR * i, 2 * _UNR), a_total(2 * _UNR), 0.0, t_end)])
    return result[0]

  jax.lax.fori_loop(0, n_main, main_body, mem0[...].astype(_F32))
  outb_copy(n_main - 1).start()

  cp_woa.wait()

  def outa_copy(q):
    t0 = pl.multiple_of(q * 128, 128)
    return pltpu.make_async_copy(
        outa.at[pl.ds(t0, 128), :], out_hbm.at[pl.ds(t0, 128), pl.ds(0, _D)], sem_outa)

  def outp_body(i, carry):
    for u in range(_TB // 128):
      q = i * (_TB // 128) + u
      o = jnp.concatenate([ot[g, q].T for g in range(_NG)], axis=1)
      t0 = pl.multiple_of(q * 128, 128)
      outa[pl.ds(t0, 128), :] = jnp.dot(
          o, woa[...], preferred_element_type=_F32).astype(_BF)
      outa_copy(q).start()
    return carry

  jax.lax.fori_loop(0, _NTB, outp_body, 0)

  def wait_a(i, carry):
    outa_copy(i).wait()
    return carry

  jax.lax.fori_loop(0, _NT, wait_a, 0)

  def wait_b(s, carry):
    outb_copy(s).wait()
    return carry

  jax.lax.fori_loop(0, n_main, wait_b, 0)


@jax.jit
def pallas_concat_heads__softmax_full_mha__memory_aug_recurrent_mem_tr__prompt_kernel(
    A_x: jax.Array,
    A_wqkv: jax.Array,
    A_wo: jax.Array,
    B_x: jax.Array,
    B_mem0: jax.Array,
    B_Wq: jax.Array,
    B_Wk: jax.Array,
    B_Wv: jax.Array,
    B_Wo: jax.Array,
    B_seg_len=_SEG,
):
  del B_seg_len
  vmem = pltpu.VMEM
  dma = pltpu.SemaphoreType.DMA
  scratch = [
      vmem((_SEQ, _D), _BF),
      vmem(((3 * _NP + 3 * _HB) * _D, 128), _BF),
      vmem((_D, _D), _BF),
      vmem((_SEQ, _D), _BF),
      vmem((_M, _D), _BF),
      vmem((_D // 128, _HB * _DHB, 128), _BF),
      vmem((2, 3, 2, _D, 128), jnp.uint32),
      vmem((_NG, _SEQ, 128), _BF),
      vmem((_NG, _NT, 128, 128), _BF),
      vmem((_NG, _NT, 128, 128), _BF),
      vmem((_NG, _NT, 128, 128), _BF),
      vmem((4, _SEQ, 128), _F32),
      vmem((4, 8, 128), _F32),
      vmem((_SEQ, _D), _BF),
      vmem((_SEQ, _D), _BF),
      vmem((_HB, _L, _DHB), _F32),
      vmem((_HB, _L, _DHB), _BF),
      vmem((_HB, _L, _DHB), _BF),
      vmem((_HB, _L, _L), _F32),
      vmem((_L, _HB * _DHB), _F32),
      dma((6,)),
      dma((_NTB,)),
      dma((_NTB,)),
      dma((2, 3, 2)),
      dma((_D // 128,)),
      dma(()),
      dma(()),
  ]
  any_spec = pl.BlockSpec(memory_space=pl.ANY)
  out = pl.pallas_call(
      _kernel,
      out_shape=jax.ShapeDtypeStruct((_SEQ, 2 * _D), _BF),
      in_specs=[any_spec] * 9,
      out_specs=any_spec,
      scratch_shapes=scratch,
      compiler_params=pltpu.CompilerParams(vmem_limit_bytes=112 * 1024 * 1024),
      name="fused_mha_rmt",
  )(
      A_x.reshape(_SEQ, _D),
      A_wqkv,
      A_wo,
      B_x.reshape(_SEQ, _D),
      B_mem0.reshape(_M, _D),
      B_Wq,
      B_Wk,
      B_Wv,
      B_Wo.reshape(_HB * _DHB, _D),
  )
  return out.reshape(1, _SEQ, 2 * _D)
```

```python
import math

import numpy as np

import jax
import jax.numpy as jnp
import jax.experimental.pallas as pl
import jax.experimental.pallas.tpu as pltpu

_BF = jnp.bfloat16
_F32 = jnp.float32

_SEQ = 2048
_D = 1024
_HA = 32
_DHA = _D // _HA
_NG = _D // 128
_NT = _SEQ // 128
_KB = 128
_LAG = 2
_SKEW = 1
_HB = 32
_DHB = 128
_M = 8
_SEG = 32
_L = _M + _SEG
_NSEG = _SEQ // _SEG
_GB = 8
_UNR = 2
_TB = 256
_NTB = _SEQ // _TB
_RD = 128
_QO = 4
_NP = _D // 128

_QSCALE = (_DHA ** -0.5) * math.log2(math.e)
_BSCALE = _DHB ** -0.5
_LOG2E = math.log2(math.e)
_HI_MASK = np.uint32(0xFFFF0000)


def _interleave(streams):
  gens = [s[0] for s in streams]
  prog = [0.0] * len(gens)
  alive = [True] * len(gens)

  def pos(k):
    st = streams[k]
    lo, hi = (st[2], st[3]) if len(st) > 2 else (0.0, 1.0)
    return lo + (hi - lo) * prog[k] / st[1]

  while any(alive):
    i = min((k for k in range(len(gens)) if alive[k]), key=pos)
    try:
      prog[i] += next(gens[i])
    except StopIteration:
      alive[i] = False


def _kernel(
    xa_hbm, wqkv_hbm, woa_hbm, xb_hbm, mem0_hbm, wq_hbm, wk_hbm, wv_hbm, wob_hbm,
    out_hbm,
    xa, wall, woa, xb, mem0, wob, raw,
    kk, qt, vt, ot, s_scr, m_scr, outa, outb,
    q_scr, k_scr, v_scr, p_scr, o_scr,
    sem_in, sem_x, sem_xb, sem_raw, sem_wob, sem_outa, sem_outb,
):
  def xa_copy(i):
    t0 = pl.multiple_of(i * _TB, _TB)
    return pltpu.make_async_copy(
        xa_hbm.at[pl.ds(t0, _TB)], xa.at[pl.ds(t0, _TB)], sem_x.at[i])

  def wa_copies(p):
    return [
        pltpu.make_async_copy(
            wqkv_hbm.at[:, pl.ds((p * _NP + n) * 128, 128)],
            wall.at[pl.ds((p * _NP + n) * _D, _D), :], sem_in.at[p])
        for n in range(_NP)
    ]

  def wa_start(p):
    for c in wa_copies(p):
      c.start()

  def wa_wait(p):
    for c in wa_copies(p):
      c.wait()

  def wa_panel(n):
    return wall[n * _D:(n + 1) * _D, :]

  def wb_rows(t, hd, r, n):
    start = (3 * _NP + t * _HB + hd) * _D + r
    if isinstance(start, int):
      return pl.ds(start, n)
    return pl.ds(pl.multiple_of(start, _RD), n)

  def xb_copy(i):
    r0 = i * _TB if isinstance(i, int) else pl.multiple_of(i * _TB, _TB)
    return pltpu.make_async_copy(
        xb_hbm.at[pl.ds(r0, _TB)], xb.at[pl.ds(r0, _TB)], sem_xb.at[i])

  cp_woa = pltpu.make_async_copy(woa_hbm, woa, sem_in.at[4])
  cp_mem = pltpu.make_async_copy(mem0_hbm, mem0, sem_in.at[5])

  def wob_copy(n):
    n0 = n * 128 if isinstance(n, int) else pl.multiple_of(n * 128, 128)
    return pltpu.make_async_copy(
        wob_hbm.at[:, pl.ds(n0, 128)], wob.at[n], sem_wob.at[n])

  wb_u32 = tuple(w.bitcast(jnp.uint32) for w in (wq_hbm, wk_hbm, wv_hbm))

  def raw_copy(i, slot, t, c):
    return pltpu.make_async_copy(
        wb_u32[t].at[:, 2 * i + c, :], raw.at[slot, t, c], sem_raw.at[slot, t, c])

  def raw_start(i, slot):
    for t in range(3):
      for c in range(2):
        raw_copy(i, slot, t, c).start()

  def raw_wait(slot):
    for t in range(3):
      for c in range(2):
        raw_copy(0, slot, t, c).wait()

  def proj_stream(i, first=False):
    t0 = pl.multiple_of(i * _TB, _TB)
    x = xa[pl.ds(t0, _TB), :]
    for part in (0, 2, 1):
      if first:
        wa_wait(part)
        if part == 0:
          wa_start(1)
          xa_copy(1).start()
          raw_start(0, 0)
        if part == 2:
          cp_mem.start()
          wob_copy(0).start()
          xb_copy(0).start()
      for g in range(_NP):
        y = jnp.dot(x, wa_panel(part * _NP + g), preferred_element_type=_F32)
        if part == 0:
          y = y * _QSCALE
        y = y.astype(_BF)
        if part == 1:
          kk[g, pl.ds(t0, _TB), :] = y
        else:
          dst = qt if part == 0 else vt
          for u in range(_TB // 128):
            dst[g, i * (_TB // 128) + u] = y[u * 128:(u + 1) * 128, :].T
        yield 1.0
  proj_total = 3 * _NP

  def relayout_stream(i, slot):
    for t in range(3):
      for c in range(2):
        for d in range(0, _D, _RD):
          w = raw[slot, t, c, d:d + _RD, :]
          lo = pltpu.bitcast(w << 16, _F32).astype(_BF)
          hi = pltpu.bitcast(w & _HI_MASK, _F32).astype(_BF)
          wall[wb_rows(t, 4 * i + 2 * c, d, _RD), :] = lo
          wall[wb_rows(t, 4 * i + 2 * c + 1, d, _RD), :] = hi
          yield 1.0
  relayout_total = 3 * 2 * (_D // _RD)

  xa_copy(0).start()
  wa_start(0)
  xa_copy(0).wait()
  wa_start(2)
  for _ in proj_stream(0, first=True):
    pass

  def proj_body(i, carry):
    slot = i % 2
    raw_start(i, slot)

    @pl.when(i + 1 < _NTB)
    def _():
      xa_copy(i + 1).start()

    wob_copy(i).start()
    xb_copy(i).start()
    xa_copy(i).wait()
    raw_wait(1 - slot)
    _interleave([(proj_stream(i), proj_total),
                 (relayout_stream(i - 1, 1 - slot), relayout_total)])
    return carry

  jax.lax.fori_loop(1, _NTB, proj_body, 0)
  cp_woa.start()

  nc = _SEQ // _KB
  nit = _NG * _NT

  def q_stationary(g, q, j):
    parts = [
        qt[g, q, 32 * j:32 * j + 32, :] if t == j else jnp.zeros((32, 128), _BF)
        for t in range(4)
    ]
    return jnp.concatenate(parts, axis=0)

  def pass1_chunk(g, qs, buf, c, m):
    s = jnp.dot(kk[g, c * _KB:(c + 1) * _KB, :], qs, preferred_element_type=_F32)
    s_scr[buf, c * _KB:(c + 1) * _KB, :] = s
    mm = s.reshape(_KB // 8, 8, 128).max(axis=0)
    return mm if m is None else jnp.maximum(m, mm)

  def pass2_chunk(g, j, buf, c, m, l, acc):
    s = s_scr[buf, c * _KB:(c + 1) * _KB, :]
    p3 = jnp.exp2(s.reshape(_KB // 8, 8, 128) - m[None])
    ls = p3.sum(axis=0)
    p = p3.reshape(_KB, 128).astype(_BF)
    v = vt[g, c, 32 * j:32 * j + 32, :]
    pv = jnp.dot(v, p, preferred_element_type=_F32)
    return (ls if l is None else l + ls), (pv if acc is None else acc + pv)

  def col_max(m):
    return jnp.broadcast_to(jnp.max(m, axis=0, keepdims=True), (8, 128))

  def a_prologue():
    for j in range(_LAG):
      qs = q_stationary(0, 0, j)
      m = None
      for c in range(nc):
        m = pass1_chunk(0, qs, j, c, m)
        yield 1.0
      m_scr[j] = col_max(m)

  raw_wait((_NTB - 1) % 2)
  _interleave([(a_prologue(), _LAG * nc),
               (relayout_stream(_NTB - 1, (_NTB - 1) % 2), relayout_total)])

  def a_stream(it0, n_it):
    for ii in range(n_it):
      it = it0 + ii
      g, q = it // _NT, it % _NT
      itn = jnp.minimum(it + 1, nit - 1)
      gn, qn = itn // _NT, itn % _NT
      for j in range(4):
        jn = (j + _LAG) % 4
        g1, q1 = (g, q) if j + _LAG < 4 else (gn, qn)
        qs = q_stationary(g1, q1, jn)
        mcur = m_scr[j]
        mn = l = acc = None
        c1 = c2 = 0
        for t in range(nc + _SKEW):
          if c2 < nc:
            l, acc = pass2_chunk(g, j, j, c2, mcur, l, acc)
            c2 += 1
            yield _KB / 16.0
            if c2 == nc:
              lt = jnp.sum(l, axis=0, keepdims=True)
              ot[g, q, 32 * j:32 * j + 32, :] = (acc * (1.0 / lt)).astype(_BF)
          if t >= _SKEW and c1 < nc:
            mn = pass1_chunk(g1, qs, jn, c1, mn)
            c1 += 1
            yield _KB / 4.0
        m_scr[jn] = col_max(mn)

  def a_total(n_it):
    return n_it * 4 * nc * (_KB / 4.0 + _KB / 16.0)

  cp_mem.wait()
  for i in range(_NTB):
    xb_copy(i).wait()
  for n in range(_D // 128):
    wob_copy(n).wait()

  row = jax.lax.broadcasted_iota(jnp.int32, (_L, _L), 0)
  col = jax.lax.broadcasted_iota(jnp.int32, (_L, _L), 1)
  mask = (row < _M) | (row >= col)

  n_main = _NSEG // _UNR
  ob_rows = _UNR * _SEG

  def outb_copy(i):
    r0 = pl.multiple_of(i * ob_rows, ob_rows)
    return pltpu.make_async_copy(
        outb.at[pl.ds(r0, ob_rows), :], out_hbm.at[pl.ds(r0, ob_rows), pl.ds(_D, _D)], sem_outb)

  def b_stream(s, mem, result):
    r0 = pl.multiple_of(s * _SEG, _SEG)
    xs = xb[pl.ds(r0, _SEG), :].astype(_F32)
    h = jnp.concatenate([mem, xs], axis=0)

    def proj(hd):
      q = jnp.dot(h, wall[wb_rows(0, hd, 0, _D), :], preferred_element_type=_F32)
      q_scr[hd] = q
      yield 80.0
      k_scr[hd] = jnp.dot(h, wall[wb_rows(1, hd, 0, _D), :], preferred_element_type=_F32).astype(_BF)
      yield 80.0
      v_scr[hd] = jnp.dot(h, wall[wb_rows(2, hd, 0, _D), :], preferred_element_type=_F32).astype(_BF)
      yield 80.0

    def scores(hd):
      sc = jax.lax.dot_general(
          q_scr[hd], k_scr[hd], (((1,), (1,)), ((), ())),
          preferred_element_type=_F32) * (_BSCALE * _LOG2E)
      sc = jnp.where(mask, sc, -1e9 * _LOG2E)
      m = jnp.max(sc, axis=-1, keepdims=True)
      p = jnp.exp2(sc - m)
      l = jnp.sum(p, axis=-1, keepdims=True)
      r = pl.reciprocal(l, approx=True)
      r = r * (2.0 - l * r)
      p = p * r
      p_scr[hd] = p
      yield 12.0

    def pv(hd):
      o = jnp.dot(p_scr[hd], v_scr[hd], preferred_element_type=_F32)
      o_scr[:, hd * _DHB:(hd + 1) * _DHB] = o
      yield 12.0

    accs = [None] * (_D // 128)

    def wo_part(gi):
      sl = slice(gi * _GB * _DHB, (gi + 1) * _GB * _DHB)
      for n in range(_D // 128):
        d = jnp.dot(o_scr[:, sl], wob[n, sl, :], preferred_element_type=_F32)
        accs[n] = d if accs[n] is None else accs[n] + d
        yield 10.0 * _GB

    ng = _HB // _GB
    for t in range(ng + 3):
      if t < ng:
        for hd in range(t * _GB, (t + 1) * _GB):
          yield from proj(hd)
      if 0 <= t - 1 < ng:
        for hd in range((t - 1) * _GB, t * _GB):
          yield from scores(hd)
      if 0 <= t - 2 < ng:
        for hd in range((t - 2) * _GB, (t - 1) * _GB):
          yield from pv(hd)
      if 0 <= t - 3 < ng:
        yield from wo_part(t - 3)
    out = jnp.concatenate(accs, axis=1)
    outb[pl.ds(r0, _SEG), :] = out[_M:].astype(_BF)
    result.append(out[:_M])
  b_total = _HB * (240.0 + 24.0) + 2560.0

  def b_multi(s0, mem, result):
    for u in range(_UNR):
      r = []
      yield from b_stream(s0 + u, mem, r)
      mem = r[0]
    result.append(mem)

  def main_body(i, mem):
    @pl.when(i > 0)
    def _():
      outb_copy(i - 1).start()

    result = []
    t_end = _UNR * (b_total + a_total(2))
    _interleave([(b_multi(i * _UNR, mem, result), _UNR * b_total, 300.0, t_end),
                 (a_stream(2 * _UNR * i, 2 * _UNR), a_total(2 * _UNR), 0.0, t_end)])
    return result[0]

  jax.lax.fori_loop(0, n_main, main_body, mem0[...].astype(_F32))
  outb_copy(n_main - 1).start()

  cp_woa.wait()

  def outa_copy(q):
    t0 = pl.multiple_of(q * 128, 128)
    return pltpu.make_async_copy(
        outa.at[pl.ds(t0, 128), :], out_hbm.at[pl.ds(t0, 128), pl.ds(0, _D)], sem_outa)

  def outp_body(i, carry):
    for u in range(_QO):
      q = i * _QO + u
      o = jnp.concatenate([ot[g, q].T for g in range(_NG)], axis=1)
      t0 = pl.multiple_of(q * 128, 128)
      outa[pl.ds(t0, 128), :] = jnp.dot(
          o, woa[...], preferred_element_type=_F32).astype(_BF)
      outa_copy(q).start()
    return carry

  jax.lax.fori_loop(0, _NT // _QO, outp_body, 0)

  def wait_a(i, carry):
    outa_copy(i).wait()
    return carry

  jax.lax.fori_loop(0, _NT, wait_a, 0)

  def wait_b(s, carry):
    outb_copy(s).wait()
    return carry

  jax.lax.fori_loop(0, n_main, wait_b, 0)


@jax.jit
def pallas_concat_heads__softmax_full_mha__memory_aug_recurrent_mem_tr__prompt_kernel(
    A_x: jax.Array,
    A_wqkv: jax.Array,
    A_wo: jax.Array,
    B_x: jax.Array,
    B_mem0: jax.Array,
    B_Wq: jax.Array,
    B_Wk: jax.Array,
    B_Wv: jax.Array,
    B_Wo: jax.Array,
    B_seg_len=_SEG,
):
  del B_seg_len
  vmem = pltpu.VMEM
  dma = pltpu.SemaphoreType.DMA
  scratch = [
      vmem((_SEQ, _D), _BF),
      vmem(((3 * _NP + 3 * _HB) * _D, 128), _BF),
      vmem((_D, _D), _BF),
      vmem((_SEQ, _D), _BF),
      vmem((_M, _D), _BF),
      vmem((_D // 128, _HB * _DHB, 128), _BF),
      vmem((2, 3, 2, _D, 128), jnp.uint32),
      vmem((_NG, _SEQ, 128), _BF),
      vmem((_NG, _NT, 128, 128), _BF),
      vmem((_NG, _NT, 128, 128), _BF),
      vmem((_NG, _NT, 128, 128), _BF),
      vmem((4, _SEQ, 128), _F32),
      vmem((4, 8, 128), _F32),
      vmem((_SEQ, _D), _BF),
      vmem((_SEQ, _D), _BF),
      vmem((_HB, _L, _DHB), _F32),
      vmem((_HB, _L, _DHB), _BF),
      vmem((_HB, _L, _DHB), _BF),
      vmem((_HB, _L, _L), _F32),
      vmem((_L, _HB * _DHB), _F32),
      dma((6,)),
      dma((_NTB,)),
      dma((_NTB,)),
      dma((2, 3, 2)),
      dma((_D // 128,)),
      dma(()),
      dma(()),
  ]
  any_spec = pl.BlockSpec(memory_space=pl.ANY)
  out = pl.pallas_call(
      _kernel,
      out_shape=jax.ShapeDtypeStruct((_SEQ, 2 * _D), _BF),
      in_specs=[any_spec] * 9,
      out_specs=any_spec,
      scratch_shapes=scratch,
      compiler_params=pltpu.CompilerParams(vmem_limit_bytes=112 * 1024 * 1024),
      name="fused_mha_rmt",
  )(
      A_x.reshape(_SEQ, _D),
      A_wqkv,
      A_wo,
      B_x.reshape(_SEQ, _D),
      B_mem0.reshape(_M, _D),
      B_Wq,
      B_Wk,
      B_Wv,
      B_Wo.reshape(_HB * _DHB, _D),
  )
  return out.reshape(1, _SEQ, 2 * _D)
```

```python
import math

import numpy as np

import jax
import jax.numpy as jnp
import jax.experimental.pallas as pl
import jax.experimental.pallas.tpu as pltpu

_BF = jnp.bfloat16
_F32 = jnp.float32

_SEQ = 2048
_D = 1024
_HA = 32
_DHA = _D // _HA
_NG = _D // 128
_NT = _SEQ // 128
_KB = 128
_LAG = 2
_SKEW = 1
_HB = 32
_DHB = 128
_M = 8
_SEG = 32
_L = _M + _SEG
_NSEG = _SEQ // _SEG
_GB = 8
_UNR = 2
_TB = 256
_NTB = _SEQ // _TB
_RD = 16
_CH = 144
_QO = 4
_NP = _D // 128

_QSCALE = (_DHA ** -0.5) * math.log2(math.e)
_BSCALE = _DHB ** -0.5
_LOG2E = math.log2(math.e)
_HI_MASK = np.uint32(0xFFFF0000)


def _interleave(streams):
  gens = [s[0] for s in streams]
  prog = [0.0] * len(gens)
  alive = [True] * len(gens)

  def pos(k):
    st = streams[k]
    lo, hi = (st[2], st[3]) if len(st) > 2 else (0.0, 1.0)
    return lo + (hi - lo) * prog[k] / st[1]

  while any(alive):
    i = min((k for k in range(len(gens)) if alive[k]), key=pos)
    try:
      prog[i] += next(gens[i])
    except StopIteration:
      alive[i] = False


def _kernel(
    xa_hbm, wqkv_hbm, woa_hbm, xb_hbm, mem0_hbm, wq_hbm, wk_hbm, wv_hbm, wob_hbm,
    out_hbm,
    xa, wall, woa, xb, mem0, wob, raw,
    kk, qt, vt, ot, s_scr, m_scr, outa, outb,
    q_scr, k_scr, v_scr, p_scr, o_scr,
    sem_in, sem_x, sem_xb, sem_raw, sem_wob, sem_outa, sem_outb,
):
  def xa_copy(i):
    t0 = pl.multiple_of(i * _TB, _TB)
    return pltpu.make_async_copy(
        xa_hbm.at[pl.ds(t0, _TB)], xa.at[pl.ds(t0, _TB)], sem_x.at[i])

  def wa_copies(p):
    return [
        pltpu.make_async_copy(
            wqkv_hbm.at[:, pl.ds((p * _NP + n) * 128, 128)],
            wall.at[pl.ds((p * _NP + n) * _D, _D), :], sem_in.at[p])
        for n in range(_NP)
    ]

  def wa_start(p):
    for c in wa_copies(p):
      c.start()

  def wa_wait(p):
    for c in wa_copies(p):
      c.wait()

  def wa_panel(n):
    return wall[n * _D:(n + 1) * _D, :]

  def wb_rows(t, hd, r, n):
    start = (3 * _NP + t * _HB + hd) * _D + r
    if isinstance(start, int):
      return pl.ds(start, n)
    return pl.ds(pl.multiple_of(start, _RD), n)

  def xb_copy(i):
    r0 = i * _TB if isinstance(i, int) else pl.multiple_of(i * _TB, _TB)
    return pltpu.make_async_copy(
        xb_hbm.at[pl.ds(r0, _TB)], xb.at[pl.ds(r0, _TB)], sem_xb.at[i])

  cp_woa = pltpu.make_async_copy(woa_hbm, woa, sem_in.at[4])
  cp_mem = pltpu.make_async_copy(mem0_hbm, mem0, sem_in.at[5])

  def wob_copy(n):
    n0 = n * 128 if isinstance(n, int) else pl.multiple_of(n * 128, 128)
    return pltpu.make_async_copy(
        wob_hbm.at[:, pl.ds(n0, 128)], wob.at[n], sem_wob.at[n])

  wb_hbm = (wq_hbm, wk_hbm, wv_hbm)
  ch_last = _D - (_NTB - 1) * _CH

  def raw_copy(i, slot, t, rows):
    d0 = i * _CH if isinstance(i, int) else pl.multiple_of(i * _CH, _RD)
    return pltpu.make_async_copy(
        wb_hbm[t].at[pl.ds(d0, rows)], raw.at[slot, t, pl.ds(0, rows)], sem_raw.at[slot, t])

  def raw_start(i, slot, rows=_CH):
    for t in range(3):
      raw_copy(i, slot, t, rows).start()

  def raw_wait(slot, rows=_CH):
    for t in range(3):
      raw_copy(0, slot, t, rows).wait()

  def proj_stream(i, first=False):
    t0 = pl.multiple_of(i * _TB, _TB)
    x = xa[pl.ds(t0, _TB), :]
    for part in (0, 2, 1):
      if first:
        wa_wait(part)
        if part == 0:
          wa_start(1)
          xa_copy(1).start()
          raw_start(0, 0)
        if part == 2:
          cp_mem.start()
          wob_copy(0).start()
          xb_copy(0).start()
      for g in range(_NP):
        y = jnp.dot(x, wa_panel(part * _NP + g), preferred_element_type=_F32)
        if part == 0:
          y = y * _QSCALE
        y = y.astype(_BF)
        if part == 1:
          kk[g, pl.ds(t0, _TB), :] = y
        else:
          dst = qt if part == 0 else vt
          for u in range(_TB // 128):
            dst[g, i * (_TB // 128) + u] = y[u * 128:(u + 1) * 128, :].T
        yield 1.0
  proj_total = 3 * _NP

  sub8 = jax.lax.broadcasted_iota(jnp.int32, (8, 128), 0)

  def transpose8(vs):
    for k in (4, 2, 1):
      m = (sub8 & k) == 0
      nv = list(vs)
      for a_i in range(8):
        if a_i & k:
          continue
        a, b = vs[a_i], vs[a_i + k]
        nv[a_i] = jnp.where(m, a, pltpu.roll(b, k, 0))
        nv[a_i + k] = jnp.where(m, pltpu.roll(a, 8 - k, 0), b)
      vs = nv
    return vs

  def relayout_stream(i, slot, rows=_CH):
    for t in range(3):
      for d in range(0, rows, _RD):
        for hh in range(2):
          groups = []
          for g in range(2):
            vs = [pltpu.bitcast(raw[slot, t, d + 8 * g + s, 16 * hh:16 * hh + 16, :], jnp.uint32)
                  for s in range(8)]
            groups.append(transpose8(vs))
          for p in range(8):
            w = jnp.concatenate([groups[0][p], groups[1][p]], axis=0)
            hd = 2 * (8 * hh + p)
            wall[wb_rows(t, hd, i * _CH + d, _RD), :] = (
                pltpu.bitcast(w << 16, _F32).astype(_BF))
            wall[wb_rows(t, hd + 1, i * _CH + d, _RD), :] = (
                pltpu.bitcast(w & _HI_MASK, _F32).astype(_BF))
          yield 1.0

  def relayout_total(rows=_CH):
    return 3 * (rows // _RD) * 2

  xa_copy(0).start()
  wa_start(0)
  xa_copy(0).wait()
  wa_start(2)
  for _ in proj_stream(0, first=True):
    pass

  def proj_body(i, carry):
    slot = i % 2

    @pl.when(i + 1 < _NTB)
    def _():
      raw_start(i, slot)
      xa_copy(i + 1).start()

    @pl.when(i + 1 == _NTB)
    def _():
      raw_start(_NTB - 1, (_NTB - 1) % 2, ch_last)

    wob_copy(i).start()
    xb_copy(i).start()
    xa_copy(i).wait()
    raw_wait(1 - slot)
    _interleave([(proj_stream(i), proj_total),
                 (relayout_stream(i - 1, 1 - slot), relayout_total())])
    return carry

  jax.lax.fori_loop(1, _NTB, proj_body, 0)
  cp_woa.start()

  nc = _SEQ // _KB
  nit = _NG * _NT

  def q_stationary(g, q, j):
    parts = [
        qt[g, q, 32 * j:32 * j + 32, :] if t == j else jnp.zeros((32, 128), _BF)
        for t in range(4)
    ]
    return jnp.concatenate(parts, axis=0)

  def pass1_chunk(g, qs, buf, c, m):
    s = jnp.dot(kk[g, c * _KB:(c + 1) * _KB, :], qs, preferred_element_type=_F32)
    s_scr[buf, c * _KB:(c + 1) * _KB, :] = s
    mm = s.reshape(_KB // 8, 8, 128).max(axis=0)
    return mm if m is None else jnp.maximum(m, mm)

  def pass2_chunk(g, j, buf, c, m, l, acc):
    s = s_scr[buf, c * _KB:(c + 1) * _KB, :]
    p3 = jnp.exp2(s.reshape(_KB // 8, 8, 128) - m[None])
    ls = p3.sum(axis=0)
    p = p3.reshape(_KB, 128).astype(_BF)
    v = vt[g, c, 32 * j:32 * j + 32, :]
    pv = jnp.dot(v, p, preferred_element_type=_F32)
    return (ls if l is None else l + ls), (pv if acc is None else acc + pv)

  def col_max(m):
    return jnp.broadcast_to(jnp.max(m, axis=0, keepdims=True), (8, 128))

  def a_prologue():
    for j in range(_LAG):
      qs = q_stationary(0, 0, j)
      m = None
      for c in range(nc):
        m = pass1_chunk(0, qs, j, c, m)
        yield 1.0
      m_scr[j] = col_max(m)

  raw_wait((_NTB - 1) % 2, ch_last)
  _interleave([(a_prologue(), _LAG * nc),
               (relayout_stream(_NTB - 1, (_NTB - 1) % 2, ch_last), relayout_total(ch_last))])

  def a_stream(it0, n_it):
    for ii in range(n_it):
      it = it0 + ii
      g, q = it // _NT, it % _NT
      itn = jnp.minimum(it + 1, nit - 1)
      gn, qn = itn // _NT, itn % _NT
      for j in range(4):
        jn = (j + _LAG) % 4
        g1, q1 = (g, q) if j + _LAG < 4 else (gn, qn)
        qs = q_stationary(g1, q1, jn)
        mcur = m_scr[j]
        mn = l = acc = None
        c1 = c2 = 0
        for t in range(nc + _SKEW):
          if c2 < nc:
            l, acc = pass2_chunk(g, j, j, c2, mcur, l, acc)
            c2 += 1
            yield _KB / 16.0
            if c2 == nc:
              lt = jnp.sum(l, axis=0, keepdims=True)
              ot[g, q, 32 * j:32 * j + 32, :] = (acc * (1.0 / lt)).astype(_BF)
          if t >= _SKEW and c1 < nc:
            mn = pass1_chunk(g1, qs, jn, c1, mn)
            c1 += 1
            yield _KB / 4.0
        m_scr[jn] = col_max(mn)

  def a_total(n_it):
    return n_it * 4 * nc * (_KB / 4.0 + _KB / 16.0)

  cp_mem.wait()
  for i in range(_NTB):
    xb_copy(i).wait()
  for n in range(_D // 128):
    wob_copy(n).wait()

  row = jax.lax.broadcasted_iota(jnp.int32, (_L, _L), 0)
  col = jax.lax.broadcasted_iota(jnp.int32, (_L, _L), 1)
  mask = (row < _M) | (row >= col)

  n_main = _NSEG // _UNR
  ob_rows = _UNR * _SEG

  def outb_copy(i):
    r0 = pl.multiple_of(i * ob_rows, ob_rows)
    return pltpu.make_async_copy(
        outb.at[pl.ds(r0, ob_rows), :], out_hbm.at[pl.ds(r0, ob_rows), pl.ds(_D, _D)], sem_outb)

  def b_stream(s, mem, result):
    r0 = pl.multiple_of(s * _SEG, _SEG)
    xs = xb[pl.ds(r0, _SEG), :].astype(_F32)
    h = jnp.concatenate([mem, xs], axis=0)

    def proj(hd):
      q = jnp.dot(h, wall[wb_rows(0, hd, 0, _D), :], preferred_element_type=_F32)
      q_scr[hd] = q
      yield 80.0
      k_scr[hd] = jnp.dot(h, wall[wb_rows(1, hd, 0, _D), :], preferred_element_type=_F32).astype(_BF)
      yield 80.0
      v_scr[hd] = jnp.dot(h, wall[wb_rows(2, hd, 0, _D), :], preferred_element_type=_F32).astype(_BF)
      yield 80.0

    def scores(hd):
      sc = jax.lax.dot_general(
          q_scr[hd], k_scr[hd], (((1,), (1,)), ((), ())),
          preferred_element_type=_F32) * (_BSCALE * _LOG2E)
      sc = jnp.where(mask, sc, -1e9 * _LOG2E)
      m = jnp.max(sc, axis=-1, keepdims=True)
      p = jnp.exp2(sc - m)
      l = jnp.sum(p, axis=-1, keepdims=True)
      r = pl.reciprocal(l, approx=True)
      r = r * (2.0 - l * r)
      p = p * r
      p_scr[hd] = p
      yield 12.0

    def pv(hd):
      o = jnp.dot(p_scr[hd], v_scr[hd], preferred_element_type=_F32)
      o_scr[:, hd * _DHB:(hd + 1) * _DHB] = o
      yield 12.0

    accs = [None] * (_D // 128)

    def wo_part(gi):
      sl = slice(gi * _GB * _DHB, (gi + 1) * _GB * _DHB)
      for n in range(_D // 128):
        d = jnp.dot(o_scr[:, sl], wob[n, sl, :], preferred_element_type=_F32)
        accs[n] = d if accs[n] is None else accs[n] + d
        yield 10.0 * _GB

    ng = _HB // _GB
    for t in range(ng + 3):
      if t < ng:
        for hd in range(t * _GB, (t + 1) * _GB):
          yield from proj(hd)
      if 0 <= t - 1 < ng:
        for hd in range((t - 1) * _GB, t * _GB):
          yield from scores(hd)
      if 0 <= t - 2 < ng:
        for hd in range((t - 2) * _GB, (t - 1) * _GB):
          yield from pv(hd)
      if 0 <= t - 3 < ng:
        yield from wo_part(t - 3)
    out = jnp.concatenate(accs, axis=1)
    outb[pl.ds(r0, _SEG), :] = out[_M:].astype(_BF)
    result.append(out[:_M])
  b_total = _HB * (240.0 + 24.0) + 2560.0

  def b_multi(s0, mem, result):
    for u in range(_UNR):
      r = []
      yield from b_stream(s0 + u, mem, r)
      mem = r[0]
    result.append(mem)

  def main_body(i, mem):
    @pl.when(i > 0)
    def _():
      outb_copy(i - 1).start()

    result = []
    t_end = _UNR * (b_total + a_total(2))
    _interleave([(b_multi(i * _UNR, mem, result), _UNR * b_total, 300.0, t_end),
                 (a_stream(2 * _UNR * i, 2 * _UNR), a_total(2 * _UNR), 0.0, t_end)])
    return result[0]

  jax.lax.fori_loop(0, n_main, main_body, mem0[...].astype(_F32))
  outb_copy(n_main - 1).start()

  cp_woa.wait()

  def outa_copy(q):
    t0 = pl.multiple_of(q * 128, 128)
    return pltpu.make_async_copy(
        outa.at[pl.ds(t0, 128), :], out_hbm.at[pl.ds(t0, 128), pl.ds(0, _D)], sem_outa)

  def outp_body(i, carry):
    for u in range(_QO):
      q = i * _QO + u
      o = jnp.concatenate([ot[g, q].T for g in range(_NG)], axis=1)
      t0 = pl.multiple_of(q * 128, 128)
      outa[pl.ds(t0, 128), :] = jnp.dot(
          o, woa[...], preferred_element_type=_F32).astype(_BF)
      outa_copy(q).start()
    return carry

  jax.lax.fori_loop(0, _NT // _QO, outp_body, 0)

  def wait_a(i, carry):
    outa_copy(i).wait()
    return carry

  jax.lax.fori_loop(0, _NT, wait_a, 0)

  def wait_b(s, carry):
    outb_copy(s).wait()
    return carry

  jax.lax.fori_loop(0, n_main, wait_b, 0)


@jax.jit
def pallas_concat_heads__softmax_full_mha__memory_aug_recurrent_mem_tr__prompt_kernel(
    A_x: jax.Array,
    A_wqkv: jax.Array,
    A_wo: jax.Array,
    B_x: jax.Array,
    B_mem0: jax.Array,
    B_Wq: jax.Array,
    B_Wk: jax.Array,
    B_Wv: jax.Array,
    B_Wo: jax.Array,
    B_seg_len=_SEG,
):
  del B_seg_len
  vmem = pltpu.VMEM
  dma = pltpu.SemaphoreType.DMA
  scratch = [
      vmem((_SEQ, _D), _BF),
      vmem(((3 * _NP + 3 * _HB) * _D, 128), _BF),
      vmem((_D, _D), _BF),
      vmem((_SEQ, _D), _BF),
      vmem((_M, _D), _BF),
      vmem((_D // 128, _HB * _DHB, 128), _BF),
      vmem((2, 3, _CH, _HB, _DHB), _BF),
      vmem((_NG, _SEQ, 128), _BF),
      vmem((_NG, _NT, 128, 128), _BF),
      vmem((_NG, _NT, 128, 128), _BF),
      vmem((_NG, _NT, 128, 128), _BF),
      vmem((4, _SEQ, 128), _F32),
      vmem((4, 8, 128), _F32),
      vmem((_SEQ, _D), _BF),
      vmem((_SEQ, _D), _BF),
      vmem((_HB, _L, _DHB), _F32),
      vmem((_HB, _L, _DHB), _BF),
      vmem((_HB, _L, _DHB), _BF),
      vmem((_HB, _L, _L), _F32),
      vmem((_L, _HB * _DHB), _F32),
      dma((6,)),
      dma((_NTB,)),
      dma((_NTB,)),
      dma((2, 3)),
      dma((_D // 128,)),
      dma(()),
      dma(()),
  ]
  any_spec = pl.BlockSpec(memory_space=pl.ANY)
  out = pl.pallas_call(
      _kernel,
      out_shape=jax.ShapeDtypeStruct((_SEQ, 2 * _D), _BF),
      in_specs=[any_spec] * 9,
      out_specs=any_spec,
      scratch_shapes=scratch,
      compiler_params=pltpu.CompilerParams(vmem_limit_bytes=112 * 1024 * 1024),
      name="fused_mha_rmt",
  )(
      A_x.reshape(_SEQ, _D),
      A_wqkv,
      A_wo,
      B_x.reshape(_SEQ, _D),
      B_mem0.reshape(_M, _D),
      B_Wq,
      B_Wk,
      B_Wv,
      B_Wo.reshape(_HB * _DHB, _D),
  )
  return out.reshape(1, _SEQ, 2 * _D)
```
